```python
import jax
import jax.numpy as jnp

def _softmax(x, axis=-1):
    return jax.nn.softmax(x, axis=axis)
def _gelu(x):
    return jax.nn.gelu(x, approximate=True)
def _silu(x):
    return jax.nn.silu(x)
def _sigmoid(x):
    return jax.nn.sigmoid(x)
def _layernorm(x, axis=-1, eps=1e-5):
    m = jnp.mean(x, axis=axis, keepdims=True)
    v = jnp.var(x, axis=axis, keepdims=True)
    return (x - m) / jnp.sqrt(v + eps)
def _scatter_add(tgt, idx, src, axis=0):
    return tgt.at[idx].add(src)
def _segment_sum(src, seg, n):
    return jax.ops.segment_sum(src, seg, n)
class _Rng:
    def __init__(self, key):
        self._k = key
    def _next(self):
        self._k, sub = jax.random.split(self._k)
        return sub
    def normal(self, shape):
        return jax.random.normal(self._next(), shape, dtype=jnp.bfloat16)
    def randint(self, lo, hi, shape):
        return jax.random.randint(self._next(), shape, lo, hi, dtype=jnp.int32)
    def uniform(self, shape, lo=0.0, hi=1.0):
        return jax.random.uniform(self._next(), shape, jnp.bfloat16, lo, hi)
    def permutation(self, n):
        return jax.random.permutation(self._next(), n)


kernel_name = 'parallel_sum__linear_attn_block__moe_arch_mod__prompt'

def setup_inputs():
    _rng = _Rng(jax.random.key(int.from_bytes(__import__("os").urandom(4), "little")))
    _w = (lambda a: (lambda t: t.astype(jnp.bfloat16) if jnp.issubdtype(t.dtype, jnp.floating) else t)(jnp.asarray(a)))
    def _A_setup():
        B, S, D = 1, 2048, 1024
        return {
            "x": _w((lambda *s: _rng.normal(s) * 0.05)(B, S, D)),
            "wqkv": _w((lambda *s: _rng.normal(s) * 0.05)(D, 3 * D)),
            "wo": _w((lambda *s: _rng.normal(s) * 0.05)(D, D)),
        }
    _A_in = _A_setup()

    def _B_setup():
        B, S, D, F, C = 1, 2048, 1024, 3584, 1
        return {
            "x": _w((lambda *s: _rng.normal(s) * 0.05)(B, S, D)),
            "w_r": _w((lambda *s: _rng.normal(s) * 0.05)(D)),
            "w_gate": _w((lambda *s: _rng.normal(s) * 0.05)(D, F)),
            "w_up": _w((lambda *s: _rng.normal(s) * 0.05)(D, F)),
            "w_down": _w((lambda *s: _rng.normal(s) * 0.05)(F, D)),
        }
    _B_in = _B_setup()

    return {
        "A_x": _A_in["x"],
        "A_wqkv": _A_in["wqkv"],
        "A_wo": _A_in["wo"],
        "B_x": _B_in["x"],
        "B_w_r": _B_in["w_r"],
        "B_w_gate": _B_in["w_gate"],
        "B_w_up": _B_in["w_up"],
        "B_w_down": _B_in["w_down"],
    }

def reference(A_x, A_wqkv, A_wo, B_x, B_w_r, B_w_gate, B_w_up, B_w_down):
    def _A_ref(x, wqkv, wo):
        B, S, D = x.shape
        H = 32; Dh = D // H
        qkv = (lambda x, *d: x.transpose(*d))((x @ wqkv).reshape(B, S, 3, H, Dh), 2, 0, 3, 1, 4)
        q, k, v = qkv[0], qkv[1], qkv[2]
        phi = lambda t: jnp.where(t > 0, t + 1, jnp.exp(t)) + 1e-6
        pq, pk = phi(q), phi(k)
        kv = jnp.einsum("bhsd,bhse->bhde", pk, v)
        z = jnp.einsum("bhsd->bhd", pk)
        num = jnp.einsum("bhqd,bhde->bhqe", pq, kv)
        den = jnp.einsum("bhqd,bhd->bhq", pq, z)[..., None] + 1e-6
        o = num / den
        return (lambda x, *d: x.transpose(*d))(o, 0, 2, 1, 3).reshape(B, S, D) @ wo

    def _B_ref(x, w_r, w_gate, w_up, w_down):
        B, S, D = x.shape
        C = 1
        r = x @ w_r
        idx = jnp.argsort(-r, axis=-1)[:, :C]
        idx_e = jnp.repeat(idx.reshape(B, C, 1), D, axis=2)
        x_sel = jnp.take_along_axis(x, idx_e, axis=1)
        g = _silu(x_sel @ w_gate)
        u = x_sel @ w_up
        y = (g * u) @ w_down
        r_sel = _sigmoid(jnp.take_along_axis(r, idx, axis=1))
        y = y * r_sel.reshape(B, C, 1)
        b_off = (jnp.arange(B) * S).reshape(B, 1)
        flat_idx = (idx + b_off).reshape(B * C)
        zero = (x * 0.0).reshape(B * S, D)
        upd = _scatter_add(zero, flat_idx, y.reshape(B * C, D), axis=0)
        return x + upd.reshape(B, S, D)

    x = A_x
    xn = _layernorm(x, axis=-1)
    return x + _A_ref(xn, A_wqkv, A_wo) + _B_ref(xn, B_w_r, B_w_gate, B_w_up, B_w_down)
```

```python
import functools
import numpy as np
import jax
import jax.numpy as jnp
from jax import lax
from jax.experimental import pallas as pl
from jax.experimental.pallas import tpu as pltpu

f32, bf16, u32 = jnp.float32, jnp.bfloat16, jnp.uint32

def _E(*terms):
    m = np.zeros((2, 2), int)
    for (s, i, j) in terms:
        m[i, j] = s
    return m
ALPHA = [_E((1,0,0),(1,1,1)), _E((1,1,0),(1,1,1)), _E((1,0,0)), _E((1,1,1)), _E((1,0,0),(1,0,1)), _E((1,1,0),(-1,0,0)), _E((1,0,1),(-1,1,1))]
BETA  = [_E((1,0,0),(1,1,1)), _E((1,0,0)), _E((1,0,1),(-1,1,1)), _E((1,1,0),(-1,0,0)), _E((1,1,1)), _E((1,0,0),(1,0,1)), _E((1,1,0),(1,1,1))]
GAMMA = [_E((1,0,0),(1,1,1)), _E((1,1,0),(-1,1,1)), _E((1,0,1),(1,1,1)), _E((1,0,0),(1,1,0)), _E((-1,0,0),(1,0,1)), _E((1,1,1)), _E((1,0,0))]
def _T(c): return [m.T for m in c]

S, D, H, DH, F = 2048, 1024, 32, 32, 3584

def _split(X):
    m, n = X.shape
    return [[X[:m//2, :n//2], X[:m//2, n//2:]], [X[m//2:, :n//2], X[m//2:, n//2:]]]

def _lin(c, b):
    pos = [b[i][j] for i in range(2) for j in range(2) if c[i, j] > 0]
    neg = [b[i][j] for i in range(2) for j in range(2) if c[i, j] < 0]
    acc = pos[0]
    for t in pos[1:]: acc = acc + t
    for t in neg: acc = acc - t
    return acc

def forms(X, coef, L):
    if L == 0: return [X]
    b = _split(X)
    out = []
    for r in range(7):
        out += forms(_lin(coef[r], b), coef, L - 1)
    return out

def combine(P, coef, L):
    if L == 0: return [[P[0]]]
    n = 7 ** (L - 1); d = 2 ** (L - 1)
    sub = [combine(P[r*n:(r+1)*n], coef, L - 1) for r in range(7)]
    grid = [[None]*(2*d) for _ in range(2*d)]
    for i in range(2):
        for k in range(2):
            for i2 in range(d):
                for k2 in range(d):
                    pos = [sub[r][i2][k2] for r in range(7) if coef[r][i, k] > 0]
                    neg = [sub[r][i2][k2] for r in range(7) if coef[r][i, k] < 0]
                    acc = pos[0]
                    for t in pos[1:]: acc = acc + t
                    for t in neg: acc = acc - t
                    grid[i*d + i2][k*d + k2] = acc
    return grid

def rnd(x):
    return x.astype(bf16).astype(f32)

def phi(t):
    return jnp.where(t > 0, t + 1.0, jnp.exp(t)) + 1e-6

def layernorm(xb):
    xf = xb.astype(f32)
    mean = jnp.mean(xf, axis=-1, keepdims=True)
    mb = rnd(mean)
    d = xf - mb
    dm = mean - mb
    var = jnp.mean(d * d, axis=-1, keepdims=True) - dm * dm
    s = rnd(jnp.sqrt(rnd(rnd(var) + rnd(jnp.float32(1e-5)))))
    xn = d * (1.0 / s)
    return xf, xn

def NN(a, b): return jnp.dot(a, b, preferred_element_type=f32)
def NT(a, b): return lax.dot_general(a, b, (((1,), (1,)), ((), ())), preferred_element_type=f32)
def TN(a, b): return lax.dot_general(a, b, (((0,), (0,)), ((), ())), preferred_element_type=f32)

def pack(x):
    return pltpu.bitcast(x.astype(bf16), u32)
def unpack(x):
    return pltpu.bitcast(x, bf16)

def make_kernel(L, TM):
    NB = S // TM
    R = 7 ** L; d = 2 ** L
    tm = TM // d
    dd = D // d
    def kernel(x_hbm, wqkv_hbm, wo_hbm, wr_hbm, wg_hbm, wu_hbm, wd_hbm, out_hbm,
               x_v, wq_v, wk_v, wv_v, wo_v, wr_v, wg_v, wu_v, wd_v,
               res, xf, pkf, wkf, wqtf, of, mf, zcol, out_v, sems):
        nsem = [0]
        def copy(src, dst):
            i = nsem[0]; nsem[0] += 1
            return pltpu.make_async_copy(src, dst, sems.at[i])
        cx = [copy(x_hbm.at[pl.ds(b*TM, TM), :], x_v.at[pl.ds(b*TM, TM), :]) for b in range(NB)]
        cwq = copy(wqkv_hbm.at[:, pl.ds(0, D)], wq_v)
        cwk = copy(wqkv_hbm.at[:, pl.ds(D, D)], wk_v)
        cwv = copy(wqkv_hbm.at[:, pl.ds(2*D, D)], wv_v)
        cwo = copy(wo_hbm, wo_v)
        cwr = copy(wr_hbm, wr_v)
        cwg = copy(wg_hbm, wg_v); cwu = copy(wu_hbm, wu_v); cwd = copy(wd_hbm, wd_v)
        cout = [copy(out_v.at[pl.ds(b*TM, TM), :], out_hbm.at[pl.ds(b*TM, TM), :]) for b in range(NB)]

        cx[0].start(); cwk.start(); cwr.start()

        st = {}
        st['m'] = jnp.full((1, 1), -jnp.inf, f32)
        st['i'] = jnp.zeros((1, 1), f32)
        def ln_block(b):
            xf32, xn = layernorm(x_v[pl.ds(b*TM, TM), :])
            res[pl.ds(b*TM, TM), :] = xf32 + xn
            fs = forms(xn, ALPHA, L)
            for r in range(R):
                xf.at[r][pl.ds(b*(tm//2), tm//2), :] = pack(fs[r])
            wr = wr_v[...].astype(f32)
            acc = None
            for j in range(D // 128):
                t = xn[:, j*128:(j+1)*128] * wr[j:j+1, :]
                acc = t if acc is None else acc + t
            rr = rnd(jnp.sum(acc, axis=-1, keepdims=True))
            mb_ = jnp.max(rr, axis=0, keepdims=True)
            rows = lax.broadcasted_iota(jnp.int32, (TM, 1), 0).astype(f32) + float(b*TM)
            ib_ = jnp.min(jnp.where(rr == mb_, rows, float(S)), axis=0, keepdims=True)
            take = mb_ > st['m']
            st['i'] = jnp.where(take, ib_, st['i'])
            st['m'] = jnp.where(take, mb_, st['m'])

        def xform(r, b=None):
            if b is None: return unpack(xf.at[r][...])
            return unpack(xf.at[r][pl.ds(b*(tm//2), tm//2), :])

        st['z'] = [None] * d
        def k_block(b):
            P = [NN(xform(r, b), unpack(wkf.at[r][...])) for r in range(R)]
            g = combine(P, GAMMA, L)
            pk = [[phi(g[i][k]) for k in range(d)] for i in range(d)]
            for k in range(d):
                for i in range(d):
                    zz = jnp.sum(pk[i][k].reshape(tm // 8, 8, dd), axis=0)
                    st['z'][k] = zz if st['z'][k] is None else st['z'][k] + zz
            pkfull = jnp.concatenate([jnp.concatenate(pk[i], axis=1) for i in range(d)], axis=0) if L else pk[0][0]
            fs = forms(pkfull, GAMMA, L)
            for r in range(R):
                pkf.at[r][pl.ds(b*(tm//2), tm//2), :] = pack(fs[r])

        cx[0].wait(); cwr.wait()
        ln_block(0)
        cwk.wait()
        if NB > 1: cx[1].start()
        wf = forms(wk_v[...].astype(f32), BETA, L)
        for r in range(R): wkf.at[r][...] = pack(wf[r])
        for b in range(NB):
            if b + 1 < NB:
                cx[b+1].wait()
                if b + 2 < NB: cx[b+2].start()
            if b == 0: cwq.start()
            if b == min(1, NB-1): cwv.start(); cwo.start()
            if b == min(2, NB-1): cwg.start()
            if b == NB - 1: cwu.start(); cwd.start()
            if b + 1 < NB: ln_block(b + 1)
            k_block(b)

        zrow = jnp.concatenate([jnp.sum(st['z'][k], axis=0, keepdims=True) for k in range(d)], axis=1)
        zb = jnp.broadcast_to(rnd(zrow), (128, D))
        zcol[...] = zb.T

        cwq.wait()
        wf = forms(wq_v[...].astype(f32), BETA, L)
        for r in range(R): wqtf.at[r][...] = pltpu.bitcast(wf[r].astype(bf16).T, u32)

        def q_block(b):
            P = [NT(unpack(wqtf.at[r][...]), xform(r, b)) for r in range(R)]
            g = combine(P, _T(GAMMA), L)
            o = [[None]*d for _ in range(d)]
            for k in range(d):
                zc = zcol[pl.ds(k*dd, dd), :]
                zc = jnp.concatenate([zc] * (tm // 128), axis=1) if tm > 128 else zc
                for i in range(d):
                    pq = phi(g[k][i])
                    t = (pq * zc).reshape(dd // DH, DH, tm)
                    den = jnp.sum(t, axis=1, keepdims=True) + 1e-6
                    o[k][i] = (pq.reshape(dd // DH, DH, tm) * (1.0 / den)).reshape(dd, tm)
            ofull = jnp.concatenate([jnp.concatenate(o[k], axis=1) for k in range(d)], axis=0) if L else o[0][0]
            fs = forms(ofull, _T(ALPHA), L)
            for r in range(R):
                of.at[b, r][...] = pack(fs[r])

        q_block(0)

        P = [TN(unpack(pkf.at[r][...]), xform(r)) for r in range(R)]
        g = combine(P, _T(BETA), L)
        Gb = jnp.concatenate([jnp.concatenate(g[k], axis=1) for k in range(d)], axis=0).astype(bf16) if L else g[0][0].astype(bf16)
        cwv.wait(); cwo.wait()
        blk = lax.broadcasted_iota(jnp.int32, (128, 128), 0) // DH == lax.broadcasted_iota(jnp.int32, (128, 128), 1) // DH
        Ms = []
        for gi in range(D // 128):
            kv = NN(Gb[gi*128:(gi+1)*128, :], wv_v[:, gi*128:(gi+1)*128])
            kv = jnp.where(blk, kv, 0.0).astype(bf16)
            Ms.append(NN(kv, wo_v[gi*128:(gi+1)*128, :]))
        Mfull = jnp.concatenate(Ms, axis=0)
        wf = forms(Mfull, BETA, L)
        for r in range(R): mf.at[r][...] = pack(wf[r])

        for b in range(1, NB): q_block(b)

        idx = jnp.max(st['i']).astype(jnp.int32)
        idx = jnp.clip(idx, 0, S - 1)
        i16 = pl.multiple_of((idx // 16) * 16, 16)
        cwg.wait(); cwu.wait()
        _, xn16 = layernorm(x_v[pl.ds(i16, 16), :])
        xs = xn16.astype(bf16)
        gg = NN(xs, wg_v[...])
        uu = NN(xs, wu_v[...])
        hh = (rnd(gg) * jax.nn.sigmoid(rnd(gg)))
        hh = (rnd(hh) * rnd(uu)).astype(bf16)
        cwd.wait()
        yy = NN(hh, wd_v[...])
        yy = yy * jax.nn.sigmoid(st['m'])
        rowm = lax.broadcasted_iota(jnp.int32, (16, D), 0) == (idx - i16)
        res[pl.ds(i16, 16), :] = res[pl.ds(i16, 16), :] + jnp.where(rowm, yy, 0.0)

        for b in range(NB):
            P = [TN(unpack(of.at[b, r][...]), unpack(mf.at[r][...])) for r in range(R)]
            g = combine(P, GAMMA, L)
            for i in range(d):
                row = jnp.concatenate(g[i], axis=1) if L else g[0][0]
                o = row + res[pl.ds(b*TM + i*tm, tm), :] if L <= 1 else None
                if L <= 1:
                    out_v[pl.ds(b*TM + i*tm, tm), :] = o.astype(bf16)
            if L == 2:
                for i in range(d):
                    row = jnp.concatenate(g[i], axis=1)
                    out_v[pl.ds(b*TM + i*tm, tm), :] = (row + res[pl.ds(b*TM + i*tm, tm), :]).astype(bf16)
            cout[b].start()
        for b in range(NB): cout[b].wait()
        assert nsem[0] <= 32
    return kernel

def build(L=1, TM=512, vmem=120, flags={'XLA_TPU_EVENLY_DISTRIBUTE_CRITICAL_NODES': True}):
    NB = S // TM; R = 7**L; d = 2**L; tm = TM // d; dd = D // d
    kern = make_kernel(L, TM)
    scratch = [
        pltpu.VMEM((S, D), bf16), pltpu.VMEM((D, D), bf16), pltpu.VMEM((D, D), bf16), pltpu.VMEM((D, D), bf16), pltpu.VMEM((D, D), bf16),
        pltpu.VMEM((8, 128), bf16), pltpu.VMEM((D, F), bf16), pltpu.VMEM((D, F), bf16), pltpu.VMEM((F, D), bf16),
        pltpu.VMEM((S, D), f32),
        pltpu.VMEM((R, S // d // 2, dd), u32), pltpu.VMEM((R, S // d // 2, dd), u32),
        pltpu.VMEM((R, dd // 2, dd), u32), pltpu.VMEM((R, dd // 2, dd), u32),
        pltpu.VMEM((NB, R, dd // 2, tm), u32), pltpu.VMEM((R, dd // 2, dd), u32),
        pltpu.VMEM((D, 128), f32), pltpu.VMEM((S, D), bf16),
        pltpu.SemaphoreType.DMA((32,)),
    ]
    any_spec = pl.BlockSpec(memory_space=pl.ANY)
    @jax.jit
    def fn(A_x, A_wqkv, A_wo, B_x, B_w_r, B_w_gate, B_w_up, B_w_down):
        out = pl.pallas_call(
            kern,
            out_shape=jax.ShapeDtypeStruct((S, D), bf16),
            in_specs=[any_spec] * 7, out_specs=any_spec,
            scratch_shapes=scratch,
            compiler_params=pltpu.CompilerParams(vmem_limit_bytes=vmem * 1024 * 1024, flags=flags),
            name=f"la_moe_L{L}_TM{TM}",
        )(A_x.reshape(S, D), A_wqkv, A_wo, B_w_r.reshape(8, 128), B_w_gate, B_w_up, B_w_down)
        return out.reshape(1, S, D)
    return fn


_impl = build()


@jax.jit
def pallas_parallel_sum__linear_attn_block__moe_arch_mod__prompt_kernel(
    A_x, A_wqkv, A_wo, B_x, B_w_r, B_w_gate, B_w_up, B_w_down):
    return _impl(A_x, A_wqkv, A_wo, B_x, B_w_r, B_w_gate, B_w_up, B_w_down)
```

```python
import functools
import numpy as np
import jax
import jax.numpy as jnp
from jax import lax
from jax.experimental import pallas as pl
from jax.experimental.pallas import tpu as pltpu

f32, bf16, u32, i32 = jnp.float32, jnp.bfloat16, jnp.uint32, jnp.int32

def _E(*terms):
    m = np.zeros((2, 2), int)
    for (s, i, j) in terms:
        m[i, j] = s
    return m
ALPHA = [_E((1,0,0),(1,1,1)), _E((1,1,0),(1,1,1)), _E((1,0,0)), _E((1,1,1)), _E((1,0,0),(1,0,1)), _E((1,1,0),(-1,0,0)), _E((1,0,1),(-1,1,1))]
BETA  = [_E((1,0,0),(1,1,1)), _E((1,0,0)), _E((1,0,1),(-1,1,1)), _E((1,1,0),(-1,0,0)), _E((1,1,1)), _E((1,0,0),(1,0,1)), _E((1,1,0),(1,1,1))]
GAMMA = [_E((1,0,0),(1,1,1)), _E((1,1,0),(-1,1,1)), _E((1,0,1),(1,1,1)), _E((1,0,0),(1,1,0)), _E((-1,0,0),(1,0,1)), _E((1,1,1)), _E((1,0,0))]
def _T(c): return [m.T for m in c]
ORDER = [1, 3, 4, 2, 0, 6, 5]

S, D, H, DH, F = 2048, 1024, 32, 32, 3584
TM = 512; NB = S // TM; tm = TM // 2; dd = D // 2; R = 7

def _lin(c, b):
    pos = [b[i][j] for i in range(2) for j in range(2) if c[i, j] > 0]
    neg = [b[i][j] for i in range(2) for j in range(2) if c[i, j] < 0]
    acc = pos[0]
    for t in pos[1:]: acc = acc + t
    for t in neg: acc = acc - t
    return acc

def comb(P, coef, i, k):
    pos = [P[r] for r in range(7) if coef[r][i, k] > 0]
    neg = [P[r] for r in range(7) if coef[r][i, k] < 0]
    acc = pos[0]
    for t in pos[1:]: acc = acc + t
    for t in neg: acc = acc - t
    return acc

def rnd(x): return x.astype(bf16).astype(f32)
def phi(t): return jnp.where(t > 0, t + 1.0, jnp.exp(t)) + 1e-6
def NN(a, b): return jnp.dot(a, b, preferred_element_type=f32)
def NT(a, b): return lax.dot_general(a, b, (((1,), (1,)), ((), ())), preferred_element_type=f32)
def TN(a, b): return lax.dot_general(a, b, (((0,), (0,)), ((), ())), preferred_element_type=f32)
def pack(x): return pltpu.bitcast(x.astype(bf16), u32)
def unpack(x): return pltpu.bitcast(x, bf16)

def ln_core(xb, z=None):
    xf = xb.astype(f32)
    if z is None:
        mean = jnp.sum(xf, axis=-1, keepdims=True) * (1.0 / D)
    else:
        ps = z
        for j in range(D // 128): ps = ps + xf[:, j*128:(j+1)*128]
        mean = jnp.sum(ps, axis=-1, keepdims=True) * (1.0 / D)
    d = xf - mean
    var = jnp.sum(d * d, axis=-1, keepdims=True) * (1.0 / D)
    inv = lax.rsqrt(var + 1e-5)
    return xf, mean, d, var, inv

def mimic_inv(var):
    s = rnd(jnp.sqrt(rnd(rnd(var) + rnd(jnp.float32(1e-5)))))
    return 1.0 / s

def gate(v):
    a = jnp.broadcast_to(jnp.sum(v, axis=-1, keepdims=True), v.shape)
    u = pltpu.bitcast(a, i32)
    return jnp.where(jnp.minimum(u, 5) <= jnp.maximum(u, 3), 0.0, a)

def ozero(a):
    u = pltpu.bitcast(a, i32)
    return jnp.where(jnp.minimum(u, 5) <= jnp.maximum(u, 3), 0.0, a)

class Metro:
    def __init__(self, seed):
        u = pltpu.bitcast(seed, i32)
        self.t = jnp.where(jnp.minimum(u, 5) <= jnp.maximum(u, 3), 1.0, seed)
    def tick(self, n):
        for _ in range(n):
            self.t = jnp.broadcast_to(jnp.sum(self.t, axis=-1, keepdims=True), (8, 128)) * (1.0 / 128)
        return ozero(self.t)

def make_kernel(opt):
    prof = opt.get('prof', False)
    CH = opt.get('chunk', 32)
    pre = opt.get('prewait', False)
    waited = set()
    def W(c, name):
        if pre and id(c) in waited:
            c = opt['_dummy']()
            c.start()
        if prof:
            with jax.named_scope(name): c.wait()
        else: c.wait()
    def W2(c, name):  return W(c, name)

    def kernel(x_hbm, wqkv_hbm, wo_hbm, wr_hbm, wg_hbm, wu_hbm, wd_hbm, out_hbm,
               x_v, wq_v, wk_v, wv_v, wo_v, wr_v, wg_v, wu_v, wd_v,
               st_mean, st_inv, xf, pkf, wkf, wqtf, of, mf, zcol, out_v, xcol, hcol, dmy, sems):
        nsem = [0]
        def copy(src, dst):
            i = nsem[0]; nsem[0] += 1
            return pltpu.make_async_copy(src, dst, sems.at[i])
        cx = [copy(x_hbm.at[pl.ds(b*TM, TM), :], x_v.at[pl.ds(b*TM, TM), :]) for b in range(NB)]
        cwk = [copy(wqkv_hbm.at[pl.ds(j*dd, dd), pl.ds(D, D)], wk_v.at[pl.ds(j*dd, dd), :]) for j in range(2)]
        cwq = copy(wqkv_hbm.at[:, pl.ds(0, D)], wq_v)
        cwv = copy(wqkv_hbm.at[:, pl.ds(2*D, D)], wv_v)
        cwo = copy(wo_hbm, wo_v)
        cwr = copy(wr_hbm, wr_v)
        cwg = copy(wg_hbm, wg_v); cwu = copy(wu_hbm, wu_v); cwd = copy(wd_hbm, wd_v)

        late = [cwg, cwu, cwd, cwv, cwo] if opt.get('bvpu') else [cwv, cwo, cwg, cwu, cwd]
        allc = [cwr, cx[0], cwk[0], cwk[1], cx[1], cx[2], cx[3], cwq] + late
        nfirst = opt.get('nfirst', len(allc))
        for c in allc[:nfirst]: c.start()

        if pre:
            for c in allc:
                c.wait(); waited.add(id(c))
            dn = [0]
            def _dummy():
                dn[0] += 1
                return pltpu.make_async_copy(wr_hbm, dmy.at[pl.ds((dn[0] % 3) * 8, 8), :], sems.at[31 - (dn[0] % 3)])
            opt['_dummy'] = _dummy
        st = {}
        lane = lax.broadcasted_iota(i32, (8, 128), 1)
        st['cvar'] = [jnp.zeros((8, 128), f32) for _ in range(2)]
        st['cdot'] = [jnp.zeros((8, 128), f32) for _ in range(2)]

        def ln_chunk(b, c):
            r0 = b*TM + c*32
            z = st.get('lnz') if b in opt.get('lnchain', ()) else None
            xf32, mean, d, var, inv = ln_core(x_v[pl.ds(r0, 32), :], z)
            if (b + 1 if c == TM // 32 - 1 else b) in opt.get('lnchain', ()):
                st['lnz'] = jnp.concatenate([ozero(jnp.broadcast_to(inv[24:32], (8, 128)))] * 4, axis=0)
            xn = d * inv
            st_mean[pl.ds(r0, 32), :] = jnp.broadcast_to(mean, (32, 128))
            st_inv[pl.ds(r0, 32), :] = jnp.broadcast_to(inv, (32, 128))
            X = [[xn[:16, :dd], xn[:16, dd:]], [xn[16:, :dd], xn[16:, dd:]]]
            for r in range(R):
                xf[pl.ds(r*(S//4) + b*(tm//2) + c*8, 8), :] = pack(_lin(ALPHA[r], X))
            wr = st['wr']
            acc = None
            for j in range(D // 128):
                t = d[:, j*128:(j+1)*128] * wr[j:j+1, :]
                acc = t if acc is None else acc + t
            dot = jnp.sum(acc, axis=-1, keepdims=True)
            for g in range(4):
                gi = (r0 // 8) + g
                sel = lane == (gi % 128)
                st['cvar'][gi // 128] = jnp.where(sel, var[g*8:(g+1)*8, :], st['cvar'][gi // 128])
                st['cdot'][gi // 128] = jnp.where(sel, dot[g*8:(g+1)*8, :], st['cdot'][gi // 128])

        def ln_block(b):
            for c in range(TM // 32): ln_chunk(b, c)

        def xform(r, b=None):
            if b is None: return unpack(xf[pl.ds(r*(S//4), S//4), :])
            return unpack(xf[pl.ds(r*(S//4) + b*(tm//2), tm//2), :])

        def wk_form(r):
            if r == 1: return wk_v[pl.ds(0, dd), pl.ds(0, dd)]
            if r == 4: return wk_v[pl.ds(dd, dd), pl.ds(dd, dd)]
            return unpack(wkf[pl.ds(r*(dd//2), dd//2), :])

        def prep_forms(src_ref, dst_ref, transpose=False, rs=range(7)):
            RC = 128
            for rc in range(dd // RC):
                need = sorted({(j, k) for r in rs for j in range(2) for k in range(2) if BETA[r][j, k]})
                Bq = [[None, None], [None, None]]
                for (j, k) in need: Bq[j][k] = src_ref[pl.ds(j*dd + rc*RC, RC), pl.ds(k*dd, dd)].astype(f32)
                for r in rs:
                    v = _lin(BETA[r], Bq)
                    if transpose:
                        vt = v.astype(bf16).T
                        dst_ref[pl.ds(r*(dd//2), dd//2), pl.ds(rc*RC, RC)] = pltpu.bitcast(vt, u32)
                    else:
                        dst_ref[pl.ds(r*(dd//2) + rc*(RC//2), RC//2), :] = pack(v)

        st['z'] = [None, None]
        def k_block(b, rs=None, P=None, finish=True, qorder=[(1, 0), (0, 1), (0, 0), (1, 1)]):
            P = {} if P is None else P
            for r in (ORDER if rs is None else rs):
                P[r] = NN(xform(r, b), wk_form(r))
            if not finish: return P
            pk = [[None, None], [None, None]]
            for (i, k) in qorder:
                pk[i][k] = phi(comb(P, GAMMA, i, k))
                zz = jnp.sum(pk[i][k].reshape(tm // 8, 8, dd), axis=0)
                st['z'][k] = zz if st['z'][k] is None else st['z'][k] + zz
            for r in range(R):
                pkf[pl.ds(r*(S//4) + b*(tm//2), tm//2), :] = pack(_lin(GAMMA[r], pk))

        W(cwr, 'w_wr'); W(cx[0], 'w_x0')
        nsecond = opt.get('nsecond', len(allc))
        for c in allc[nfirst:nsecond]: c.start()
        st['wr'] = wr_v[...].astype(f32)
        ln_block(0)
        if opt.get('trunc'):
            W(cwk[0], 'w_wk0'); W(cwk[1], 'w_wk1'); W(cx[1], 'w_x1'); W(cx[2], 'w_x2'); W(cx[3], 'w_x3')
            for c in [cwq] + late: c.wait()
            out_v[pl.ds(0, 512), :] = (unpack(xf[pl.ds(0, 256), :]).astype(f32).sum() + x_v[pl.ds(512, 512), :].astype(f32)).astype(bf16)
            c = copy(out_v.at[pl.ds(0, 512), :], out_hbm.at[pl.ds(0, 512), :]); c.start(); c.wait()
            return
        W(cwk[0], 'w_wk0')
        prep_forms(wk_v, wkf, rs=[5])
        P0 = k_block(0, rs=[1, 5], finish=False)
        W(cwk[1], 'w_wk1')
        for c in allc[max(nfirst, nsecond):]: c.start()
        prep_forms(wk_v, wkf, rs=[2, 3, 0, 6])
        s0 = opt.get('split0', 2)
        rest = [4, 2, 3, 0, 6]
        P0 = k_block(0, rs=rest[:s0], P=P0, finish=False)
        W(cx[1], 'w_x1')
        ln_block(1)
        k_block(0, rs=rest[s0:], P=P0, qorder=[(0, 1), (1, 0), (1, 1), (0, 0)])
        if opt.get('mergex', False):
            W(cx[2], 'w_x2'); W(cx[3], 'w_x3')
            ln_block(2); k_block(1); ln_block(3); k_block(2)
        else:
            W(cx[2], 'w_x2'); ln_block(2); k_block(1)
            W(cx[3], 'w_x3')
            if opt.get('mq', True): W(cwq, 'w_wq')
            ln_block(3); k_block(2)
        if not opt.get('mq', True): W(cwq, 'w_wq')
        if not opt.get('bvpu'): W(cwv, 'w_wv'); W(cwo, 'w_wo')
        prep_forms(wq_v, wqtf, transpose=True)
        k_block(3)

        sub = lax.broadcasted_iota(i32, (8, 128), 0)
        rs_, ix_ = [], []
        for hlf in range(2):
            rr = rnd(st['cdot'][hlf] * mimic_inv(st['cvar'][hlf]))
            rs_.append(rr); ix_.append(((lane + hlf*128) * 8 + sub).astype(f32))
        rmax = jnp.max(jnp.maximum(rs_[0], rs_[1]), keepdims=True)
        cand = jnp.minimum(jnp.where(rs_[0] == rmax, ix_[0], float(S)), jnp.where(rs_[1] == rmax, ix_[1], float(S)))
        idxf = jnp.min(cand, keepdims=True)

        zrow = jnp.concatenate([jnp.sum(st['z'][k], axis=0, keepdims=True) for k in range(2)], axis=1)
        zcol[...] = jnp.broadcast_to(zrow, (128, D)).T

        def q_block(b):
            P = {}
            for r in ORDER:
                P[r] = NT(unpack(wqtf[pl.ds(r*(dd//2), dd//2), :]), xform(r, b))
            o = [[None, None], [None, None]]
            for (i, k) in [(1, 0), (0, 1), (0, 0), (1, 1)]:
                zc = zcol[pl.ds(k*dd, dd), :]
                zc = jnp.concatenate([zc] * (tm // 128), axis=1)
                pq = phi(comb(P, GAMMA, i, k))
                t = (pq * zc).reshape(dd // DH, DH, tm)
                den = jnp.sum(t, axis=1, keepdims=True) + 1e-6
                o[k][i] = (pq.reshape(dd // DH, DH, tm) * (1.0 / den)).reshape(dd, tm)
            for r in range(R):
                of[pl.ds((b*R + r)*(dd//2), dd//2), :] = pack(_lin(ALPHA[r].T, o))

        nq_pre = opt.get('nq_pre', 1)
        for b in range(nq_pre): q_block(b)

        def b_path():
            idx = jnp.clip(jnp.max(idxf).astype(i32), 0, S - 1)
            i16 = pl.multiple_of((idx // 16) * 16, 16)
            W(cwg, 'w_wg'); W(cwu, 'w_wu'); W(cwd, 'w_wd')
            _, _, d16, var16, inv16 = ln_core(x_v[pl.ds(i16, 16), :])
            xs = (d16 * inv16).astype(bf16)
            gg = rnd(NN(xs, wg_v[...]))
            uu = rnd(NN(xs, wu_v[...]))
            hh = (rnd(gg * jax.nn.sigmoid(gg)) * uu).astype(bf16)
            yy = NN(hh, wd_v[...]) * jax.nn.sigmoid(rmax)
            rowm = lax.broadcasted_iota(i32, (16, D), 0) == (idx - i16)
            st['yy'] = jnp.where(rowm, yy, 0.0); st['i16'] = i16


        CW = opt.get('cw', 512)
        def bv_stage0():
            idx = jnp.clip(jnp.max(idxf).astype(i32), 0, S - 1)
            i16 = pl.multiple_of((idx // 16) * 16, 16)
            x16 = x_v[pl.ds(i16, 16), :].astype(f32)
            mean = jnp.concatenate([st_mean[pl.ds(i16, 16), :]] * (D // 128), axis=1)
            inv = jnp.concatenate([st_inv[pl.ds(i16, 16), :]] * (D // 128), axis=1)
            xs = rnd((x16 - mean) * inv)
            rowm = lax.broadcasted_iota(i32, (16, D), 0) == (idx - i16)
            xrow = jnp.sum(jnp.where(rowm, xs, 0.0), axis=0, keepdims=True)
            xcol[...] = jnp.broadcast_to(xrow, (128, D)).T
            st['i16'] = i16; st['rowm'] = rowm
        def matvec(w_ref, col_ref, nrows, c0, cw, seg=None, z=None, metro=None, nt=0):
            acc = None
            for i in range(nrows // 8):
                if metro is not None and i % seg == 0:
                    z = metro.tick(nt)
                elif metro is None and seg and i % seg == 0 and i > 0:
                    z = gate(acc[:, :128])
                w = w_ref[pl.ds(8*i, 8), pl.ds(c0, cw)].astype(f32)
                xc = col_ref[pl.ds(8*i, 8), :]
                if cw > 128: xc = jnp.concatenate([xc] * (cw // 128), axis=1)
                t = w * xc
                if z is not None:
                    t = t + (jnp.concatenate([z] * (cw // 128), axis=1) if cw > 128 else z); z = None
                acc = t if acc is None else acc + t
            return acc
        def bv_stage1_serial():
            z = None
            for c in range(F // 128):
                ga = matvec(wg_v, xcol, D, c*128, 128, z=z); z = ozero(ga)
                ua = matvec(wu_v, xcol, D, c*128, 128, z=z); z = ozero(ua)
                gg = rnd(jnp.sum(ga, axis=0, keepdims=True))
                uu = rnd(jnp.sum(ua, axis=0, keepdims=True))
                hh = rnd(rnd(gg * jax.nn.sigmoid(gg)) * uu)
                hcol[pl.ds(c*128, 128), :] = jnp.broadcast_to(hh, (128, 128)).T
        def bv_stage2_serial():
            z = None; ys = []
            for n in range(D // 128):
                ya = matvec(wd_v, hcol, F, n*128, 128, z=z); z = ozero(ya)
                ys.append(jnp.sum(ya, axis=0, keepdims=True))
            st['yacc'] = ya
            yy = jnp.concatenate(ys, axis=1) * jax.nn.sigmoid(rmax)
            st['yy'] = jnp.where(st['rowm'], yy, 0.0)
        def bv_stage1():
            if opt.get('serial'): return bv_stage1_serial()
            z = None
            m1 = Metro(xcol[pl.ds(0, 8), :]) if opt.get('nt1') else None
            for c in range(F // CW):
                ga = matvec(wg_v, xcol, D, c*CW, CW, seg=opt.get('seg1'), z=z, metro=m1, nt=opt.get('nt1', 0))
                if opt.get('chain1') == 2: z = gate(ga[:, :128])
                ua = matvec(wu_v, xcol, D, c*CW, CW, seg=opt.get('seg1'), z=z, metro=m1, nt=opt.get('nt1', 0))
                if opt.get('chain1'): z = gate(ua[:, :128])
                gg = rnd(jnp.sum(ga, axis=0, keepdims=True))
                uu = rnd(jnp.sum(ua, axis=0, keepdims=True))
                hh = rnd(rnd(gg * jax.nn.sigmoid(gg)) * uu)
                for j in range(CW // 128):
                    hcol[pl.ds(c*CW + j*128, 128), :] = jnp.broadcast_to(hh[:, j*128:(j+1)*128], (128, 128)).T
        def bv_stage2():
            if opt.get('serial'): return bv_stage2_serial()
            CN = opt.get('cn', 1024)
            m2 = Metro(xcol[pl.ds(0, 8), :]) if opt.get('nt2') else None
            ys = [jnp.sum(matvec(wd_v, hcol, F, n*CN, CN, seg=opt.get('seg2'), metro=m2, nt=opt.get('nt2', 0)), axis=0, keepdims=True) for n in range(D // CN)]
            yy = jnp.concatenate(ys, axis=1) * jax.nn.sigmoid(rmax)
            st['yy'] = jnp.where(st['rowm'], yy, 0.0)

        P = {}
        n1 = opt.get('g1', 4)
        if opt.get('bvpu'):
            bv_stage0()
            W(cwg, 'w_wg'); W(cwu, 'w_wu')
            bv_stage1()
        for r in ORDER[:n1]:
            P[r] = TN(unpack(pkf[pl.ds(r*(S//4), S//4), :]), xform(r))
        if opt.get('bvpu'):
            W(cwd, 'w_wd')
            if opt.get('mv', True): W(cwv, 'w_wv'); W(cwo, 'w_wo')
            bv_stage2()
        for r in ORDER[n1:]:
            P[r] = TN(unpack(pkf[pl.ds(r*(S//4), S//4), :]), xform(r))
        if opt.get('bvpu') and not opt.get('mv', True): W(cwv, 'w_wv'); W(cwo, 'w_wo')
        if opt.get('bpos') == 'trans': b_path()
        st['kvzero'] = jnp.concatenate([ozero(st['yacc'])] * 16, axis=0) if opt.get('bvpu') and opt.get('pin', True) else 0.0
        blk = lax.broadcasted_iota(i32, (128, 128), 0) // DH == lax.broadcasted_iota(i32, (128, 128), 1) // DH
        Mq = [[None, None], [None, None]]
        for k in range(2):
            Gk = [comb(P, _T(BETA), k, j) for j in range(2)]
            Ms = []
            for gi in range(dd // 128):
                g = k*(dd//128) + gi
                Gg = jnp.concatenate([Gk[j][gi*128:(gi+1)*128, :].astype(bf16) for j in range(2)], axis=1)
                kv = NN(Gg, wv_v[:, pl.ds(g*128, 128)])
                kv = jnp.where(blk, kv, st['kvzero']).astype(bf16)
                Ms.append(NN(kv, wo_v[pl.ds(g*128, 128), :]))
            Mk = jnp.concatenate(Ms, axis=0)
            Mq[k] = [Mk[:, :dd], Mk[:, dd:]]
        for r in range(R):
            mf[pl.ds(r*(dd//2), dd//2), :] = pack(_lin(BETA[r], Mq))

        if opt.get('bpos') == 'posttrans': b_path()
        for b in range(nq_pre, NB):
            if opt.get('bpos') == f'q{b}': b_path()
            q_block(b)

        if opt.get('bpos', 'late') == 'late' and not opt.get('bvpu'): b_path()

        pend = []
        def a_piece(b, c0, nc, split_cols):
            P = {}
            for r in ORDER:
                P[r] = TN(unpack(of[pl.ds((b*R + r)*(dd//2), dd//2), pl.ds(c0*16, nc*16)]), unpack(mf[pl.ds(r*(dd//2), dd//2), :]))
            row0 = b*TM + c0*32; nrows = nc*32
            i16 = st['i16']; yy = st['yy']
            def emit(i, k):
                Aq = comb(P, GAMMA, i, k)
                for c in range(nc):
                    r0 = row0 + c*32 + i*16
                    xx = x_v[pl.ds(r0, 16), pl.ds(k*dd, dd)].astype(f32)
                    mean = jnp.concatenate([st_mean[pl.ds(r0, 16), :]] * (dd // 128), axis=1)
                    inv = jnp.concatenate([st_inv[pl.ds(r0, 16), :]] * (dd // 128), axis=1)
                    o = (Aq[c*16:(c+1)*16, :] + xx) + (xx - mean) * inv
                    out_v[pl.ds(r0, 16), pl.ds(k*dd, dd)] = o.astype(bf16)
            def patch_and_send(col0, ncol):
                off = pl.multiple_of(jnp.clip(i16 - row0, 0, nrows - 16), 16) + row0
                inb = jnp.logical_and(i16 >= row0, i16 < row0 + nrows)
                tile = out_v[pl.ds(off, 16), pl.ds(col0, ncol)].astype(f32) + jnp.where(inb, yy[:, col0:col0+ncol], 0.0)
                out_v[pl.ds(off, 16), pl.ds(col0, ncol)] = tile.astype(bf16)
                c = copy(out_v.at[pl.ds(row0, nrows), pl.ds(col0, ncol)], out_hbm.at[pl.ds(row0, nrows), pl.ds(col0, ncol)])
                c.start(); pend.append(c)
            if split_cols:
                emit(1, 0); emit(0, 1); emit(0, 0); patch_and_send(0, dd)
                emit(1, 1); patch_and_send(dd, dd)
            else:
                for (i, k) in [(1, 0), (0, 1), (0, 0), (1, 1)]: emit(i, k)
                patch_and_send(0, D)
        tail = opt.get('tail', 2)
        for b in range(NB - 1): a_piece(b, 0, 16, False)
        if tail == 0: a_piece(NB - 1, 0, 16, False)
        elif tail == 1: a_piece(NB - 1, 0, 16, True)
        elif tail == 2: a_piece(NB - 1, 0, 8, False); a_piece(NB - 1, 8, 8, True)
        elif tail == 3: a_piece(NB - 1, 0, 8, False); a_piece(NB - 1, 8, 8, False)
        for n, c in enumerate(pend): W(c, f'w_out{n}')
        assert nsem[0] <= 29
    return kernel

def build(vmem=120, flags={'XLA_TPU_EVENLY_DISTRIBUTE_CRITICAL_NODES': True}, **opt):
    kern = make_kernel(opt)
    scratch = [
        pltpu.VMEM((S, D), bf16), pltpu.VMEM((D, D), bf16), pltpu.VMEM((D, D), bf16), pltpu.VMEM((D, D), bf16), pltpu.VMEM((D, D), bf16),
        pltpu.VMEM((8, 128), bf16), pltpu.VMEM((D, F), bf16), pltpu.VMEM((D, F), bf16), pltpu.VMEM((F, D), bf16),
        pltpu.VMEM((S, 128), f32), pltpu.VMEM((S, 128), f32),
        pltpu.VMEM((R * S // 4, dd), u32), pltpu.VMEM((R * S // 4, dd), u32),
        pltpu.VMEM((R * dd // 2, dd), u32), pltpu.VMEM((R * dd // 2, dd), u32),
        pltpu.VMEM((NB * R * dd // 2, tm), u32), pltpu.VMEM((R * dd // 2, dd), u32),
        pltpu.VMEM((D, 128), f32), pltpu.VMEM((S, D), bf16), pltpu.VMEM((D, 128), f32), pltpu.VMEM((F, 128), f32), pltpu.VMEM((24, 128), bf16),
        pltpu.SemaphoreType.DMA((32,)),
    ]
    any_spec = pl.BlockSpec(memory_space=pl.ANY)
    @jax.jit
    def fn(A_x, A_wqkv, A_wo, B_x, B_w_r, B_w_gate, B_w_up, B_w_down):
        out = pl.pallas_call(
            kern,
            out_shape=jax.ShapeDtypeStruct((S, D), bf16),
            in_specs=[any_spec] * 7, out_specs=any_spec,
            scratch_shapes=scratch,
            compiler_params=pltpu.CompilerParams(vmem_limit_bytes=vmem * 1024 * 1024, flags=flags),
            name="la_moe_k3",
        )(A_x.reshape(S, D), A_wqkv, A_wo, B_w_r.reshape(8, 128), B_w_gate, B_w_up, B_w_down)
        return out.reshape(1, S, D)
    return fn


_impl = build(bvpu=True,nq_pre=3,serial=True,g1=5)


@jax.jit
def pallas_parallel_sum__linear_attn_block__moe_arch_mod__prompt_kernel(
    A_x, A_wqkv, A_wo, B_x, B_w_r, B_w_gate, B_w_up, B_w_down):
    return _impl(A_x, A_wqkv, A_wo, B_x, B_w_r, B_w_gate, B_w_up, B_w_down)
```

```python
import functools
import numpy as np
import jax
import jax.numpy as jnp
from jax import lax
from jax.experimental import pallas as pl
from jax.experimental.pallas import tpu as pltpu

f32, bf16, u32, i32 = jnp.float32, jnp.bfloat16, jnp.uint32, jnp.int32

def _E(*terms):
    m = np.zeros((2, 2), int)
    for (s, i, j) in terms:
        m[i, j] = s
    return m
ALPHA = [_E((1,0,0),(1,1,1)), _E((1,1,0),(1,1,1)), _E((1,0,0)), _E((1,1,1)), _E((1,0,0),(1,0,1)), _E((1,1,0),(-1,0,0)), _E((1,0,1),(-1,1,1))]
BETA  = [_E((1,0,0),(1,1,1)), _E((1,0,0)), _E((1,0,1),(-1,1,1)), _E((1,1,0),(-1,0,0)), _E((1,1,1)), _E((1,0,0),(1,0,1)), _E((1,1,0),(1,1,1))]
GAMMA = [_E((1,0,0),(1,1,1)), _E((1,1,0),(-1,1,1)), _E((1,0,1),(1,1,1)), _E((1,0,0),(1,1,0)), _E((-1,0,0),(1,0,1)), _E((1,1,1)), _E((1,0,0))]
def _T(c): return [m.T for m in c]
ORDER = [1, 3, 4, 2, 0, 6, 5]

S, D, H, DH, F = 2048, 1024, 32, 32, 3584
TM = 512; NB = S // TM; tm = TM // 2; dd = D // 2; R = 7

def _lin(c, b):
    pos = [b[i][j] for i in range(2) for j in range(2) if c[i, j] > 0]
    neg = [b[i][j] for i in range(2) for j in range(2) if c[i, j] < 0]
    acc = pos[0]
    for t in pos[1:]: acc = acc + t
    for t in neg: acc = acc - t
    return acc

def comb(P, coef, i, k):
    pos = [P[r] for r in range(7) if coef[r][i, k] > 0]
    neg = [P[r] for r in range(7) if coef[r][i, k] < 0]
    acc = pos[0]
    for t in pos[1:]: acc = acc + t
    for t in neg: acc = acc - t
    return acc

def rnd(x): return x.astype(bf16).astype(f32)
def phi(t): return jnp.where(t > 0, t + 1.0, jnp.exp(t)) + 1e-6
def NN(a, b): return jnp.dot(a, b, preferred_element_type=f32)
def NT(a, b): return lax.dot_general(a, b, (((1,), (1,)), ((), ())), preferred_element_type=f32)
def TN(a, b): return lax.dot_general(a, b, (((0,), (0,)), ((), ())), preferred_element_type=f32)
def pack(x): return pltpu.bitcast(x.astype(bf16), u32)
def unpack(x): return pltpu.bitcast(x, bf16)

def ln_core(xb, z=None):
    xf = xb.astype(f32)
    if z is None:
        mean = jnp.sum(xf, axis=-1, keepdims=True) * (1.0 / D)
    else:
        ps = z
        for j in range(D // 128): ps = ps + xf[:, j*128:(j+1)*128]
        mean = jnp.sum(ps, axis=-1, keepdims=True) * (1.0 / D)
    d = xf - mean
    var = jnp.sum(d * d, axis=-1, keepdims=True) * (1.0 / D)
    inv = lax.rsqrt(var + 1e-5)
    return xf, mean, d, var, inv

def mimic_inv(var):
    s = rnd(jnp.sqrt(rnd(rnd(var) + rnd(jnp.float32(1e-5)))))
    return 1.0 / s

def gate(v):
    a = jnp.broadcast_to(jnp.sum(v, axis=-1, keepdims=True), v.shape)
    u = pltpu.bitcast(a, i32)
    return jnp.where(jnp.minimum(u, 5) <= jnp.maximum(u, 3), 0.0, a)

def ozero(a):
    u = pltpu.bitcast(a, i32)
    return jnp.where(jnp.minimum(u, 5) <= jnp.maximum(u, 3), 0.0, a)

class Metro:
    def __init__(self, seed):
        u = pltpu.bitcast(seed, i32)
        self.t = jnp.where(jnp.minimum(u, 5) <= jnp.maximum(u, 3), 1.0, seed)
    def tick(self, n):
        for _ in range(n):
            self.t = jnp.broadcast_to(jnp.sum(self.t, axis=-1, keepdims=True), (8, 128)) * (1.0 / 128)
        return ozero(self.t)

def make_kernel(opt):
    LA = opt.get('LA', 1)
    prof = opt.get('prof', False)
    CH = opt.get('chunk', 32)
    pre = opt.get('prewait', False)
    waited = set()
    def W(c, name):
        if pre and id(c) in waited:
            c = opt['_dummy']()
            c.start()
        if prof:
            with jax.named_scope(name): c.wait()
        else: c.wait()
    def W2(c, name):  return W(c, name)

    def kernel(x_hbm, wqkv_hbm, wo_hbm, wr_hbm, wg_hbm, wu_hbm, wd_hbm, out_hbm,
               x_v, wq_v, wk_v, wv_v, wo_v, wr_v, wg_v, wu_v, wd_v,
               st_mean, st_inv, xf, pkf, wkf, wqtf, of, mf, zcol, out_v, xcol, hcol, dmy, ofb, sems):
        nsem = [0]
        def copy(src, dst):
            i = nsem[0]; nsem[0] += 1
            return pltpu.make_async_copy(src, dst, sems.at[i])
        NX0 = opt.get('nx0', 1); RX = TM // NX0
        cx0 = [copy(x_hbm.at[pl.ds(i*RX, RX), :], x_v.at[pl.ds(i*RX, RX), :]) for i in range(NX0)]
        cx = [None] + [copy(x_hbm.at[pl.ds(b*TM, TM), :], x_v.at[pl.ds(b*TM, TM), :]) for b in range(1, NB)]
        cwk = [copy(wqkv_hbm.at[pl.ds(j*dd, dd), pl.ds(D, D)], wk_v.at[pl.ds(j*dd, dd), :]) for j in range(2)]
        cwq = copy(wqkv_hbm.at[:, pl.ds(0, D)], wq_v)
        cwv = copy(wqkv_hbm.at[:, pl.ds(2*D, D)], wv_v)
        cwo = copy(wo_hbm, wo_v)
        cwr = copy(wr_hbm, wr_v)
        cwg = copy(wg_hbm, wg_v); cwu = copy(wu_hbm, wu_v); cwd = copy(wd_hbm, wd_v)

        late = [cwg, cwu, cwd, cwv, cwo] if opt.get('bvpu') else [cwv, cwo, cwg, cwu, cwd]
        allc = [cwr] + cx0 + [cwk[0], cwk[1], cx[1], cx[2], cx[3], cwq] + late
        nfirst = opt.get('nfirst', len(allc))
        for n_, c in enumerate(allc[:nfirst]): c.start(priority=1 if n_ >= opt.get('lowprio', 99) else 0)

        if pre:
            for c in allc:
                c.wait(); waited.add(id(c))
            dn = [0]
            def _dummy():
                dn[0] += 1
                return pltpu.make_async_copy(wr_hbm, dmy.at[pl.ds((dn[0] % 3) * 8, 8), :], sems.at[39 - (dn[0] % 3)])
            opt['_dummy'] = _dummy
        st = {}
        lane = lax.broadcasted_iota(i32, (8, 128), 1)
        st['cvar'] = [jnp.zeros((8, 128), f32) for _ in range(2)]
        st['cdot'] = [jnp.zeros((8, 128), f32) for _ in range(2)]

        def ln_chunk(b, c):
            r0 = b*TM + c*32
            z = st.get('lnz') if b in opt.get('lnchain', ()) else None
            xf32, mean, d, var, inv = ln_core(x_v[pl.ds(r0, 32), :], z)
            if (b + 1 if c == TM // 32 - 1 else b) in opt.get('lnchain', ()):
                st['lnz'] = jnp.concatenate([ozero(jnp.broadcast_to(inv[24:32], (8, 128)))] * 4, axis=0)
            xn = d * inv
            st_mean[pl.ds(r0, 32), :] = jnp.broadcast_to(mean, (32, 128))
            st_inv[pl.ds(r0, 32), :] = jnp.broadcast_to(inv, (32, 128))
            X = [[xn[:16, :dd], xn[:16, dd:]], [xn[16:, :dd], xn[16:, dd:]]]
            for r in range(R):
                xf[pl.ds(r*(S//4) + b*(tm//2) + c*8, 8), :] = pack(_lin(ALPHA[r], X))
            wr = st['wr']
            acc = None
            for j in range(D // 128):
                t = d[:, j*128:(j+1)*128] * wr[j:j+1, :]
                acc = t if acc is None else acc + t
            dot = jnp.sum(acc, axis=-1, keepdims=True)
            for g in range(4):
                gi = (r0 // 8) + g
                sel = lane == (gi % 128)
                st['cvar'][gi // 128] = jnp.where(sel, var[g*8:(g+1)*8, :], st['cvar'][gi // 128])
                st['cdot'][gi // 128] = jnp.where(sel, dot[g*8:(g+1)*8, :], st['cdot'][gi // 128])

        def ln_block(b):
            for c in range(TM // 32): ln_chunk(b, c)

        def xform(r, b=None):
            if b is None: return unpack(xf[pl.ds(r*(S//4), S//4), :])
            return unpack(xf[pl.ds(r*(S//4) + b*(tm//2), tm//2), :])

        def wk_form(r):
            if r == 1: return wk_v[pl.ds(0, dd), pl.ds(0, dd)]
            if r == 4: return wk_v[pl.ds(dd, dd), pl.ds(dd, dd)]
            return unpack(wkf[pl.ds(r*(dd//2), dd//2), :])

        def prep_forms(src_ref, dst_ref, transpose=False, rs=range(7)):
            RC = 128
            for rc in range(dd // RC):
                need = sorted({(j, k) for r in rs for j in range(2) for k in range(2) if BETA[r][j, k]})
                Bq = [[None, None], [None, None]]
                for (j, k) in need: Bq[j][k] = src_ref[pl.ds(j*dd + rc*RC, RC), pl.ds(k*dd, dd)].astype(f32)
                for r in rs:
                    v = _lin(BETA[r], Bq)
                    if transpose:
                        vt = v.astype(bf16).T
                        dst_ref[pl.ds(r*(dd//2), dd//2), pl.ds(rc*RC, RC)] = pltpu.bitcast(vt, u32)
                    else:
                        dst_ref[pl.ds(r*(dd//2) + rc*(RC//2), RC//2), :] = pack(v)

        st['z'] = [None, None]
        def k_block(b, rs=None, P=None, finish=True, qorder=[(1, 0), (0, 1), (0, 0), (1, 1)]):
            P = {} if P is None else P
            for r in (ORDER if rs is None else rs):
                P[r] = NN(xform(r, b), wk_form(r))
            if not finish: return P
            pk = [[None, None], [None, None]]
            for (i, k) in qorder:
                pk[i][k] = phi(comb(P, GAMMA, i, k))
                zz = jnp.sum(pk[i][k].reshape(tm // 8, 8, dd), axis=0)
                st['z'][k] = zz if st['z'][k] is None else st['z'][k] + zz
            for r in range(R):
                pkf[pl.ds(r*(S//4) + b*(tm//2), tm//2), :] = pack(_lin(GAMMA[r], pk))

        W(cwr, 'w_wr')
        nsecond = opt.get('nsecond', len(allc))
        st['wr'] = wr_v[...].astype(f32)
        for i in range(NX0):
            W(cx0[i], f'w_x0_{i}')
            for c in range(i*(16 // NX0), (i+1)*(16 // NX0)): ln_chunk(0, c)
        if opt.get('trunc'):
            W(cwk[0], 'w_wk0'); W(cwk[1], 'w_wk1'); W(cx[1], 'w_x1'); W(cx[2], 'w_x2'); W(cx[3], 'w_x3')
            for c in [cwq] + late: c.wait()
            out_v[pl.ds(0, 512), :] = (unpack(xf[pl.ds(0, 256), :]).astype(f32).sum() + x_v[pl.ds(512, 512), :].astype(f32)).astype(bf16)
            c = copy(out_v.at[pl.ds(0, 512), :], out_hbm.at[pl.ds(0, 512), :]); c.start(); c.wait()
            return
        W(cwk[0], 'w_wk0')
        prep_forms(wk_v, wkf, rs=[5])
        P0 = k_block(0, rs=[1, 5], finish=False)
        W(cwk[1], 'w_wk1')
        for c in allc[max(nfirst, nsecond):]: c.start()
        prep_forms(wk_v, wkf, rs=[2, 3, 0, 6])
        s0 = opt.get('split0', 2)
        rest = [4, 2, 3, 0, 6]
        P0 = k_block(0, rs=rest[:s0], P=P0, finish=False)
        W(cx[1], 'w_x1')
        ln_block(1)
        k_block(0, rs=rest[s0:], P=P0, qorder=[(0, 1), (1, 0), (1, 1), (0, 0)])
        if opt.get('mergex', False):
            W(cx[2], 'w_x2'); W(cx[3], 'w_x3')
            ln_block(2); k_block(1); ln_block(3); k_block(2)
        else:
            W(cx[2], 'w_x2'); ln_block(2); k_block(1)
            W(cx[3], 'w_x3')
            if opt.get('mq', True): W(cwq, 'w_wq')
            ln_block(3); k_block(2)
        if not opt.get('mq', True): W(cwq, 'w_wq')
        if not opt.get('bvpu'): W(cwv, 'w_wv'); W(cwo, 'w_wo')
        prep_forms(wq_v, wqtf, transpose=True)
        k_block(3)

        sub = lax.broadcasted_iota(i32, (8, 128), 0)
        rs_, ix_ = [], []
        for hlf in range(2):
            rr = rnd(st['cdot'][hlf] * mimic_inv(st['cvar'][hlf]))
            rs_.append(rr); ix_.append(((lane + hlf*128) * 8 + sub).astype(f32))
        rmax = jnp.max(jnp.maximum(rs_[0], rs_[1]), keepdims=True)
        cand = jnp.minimum(jnp.where(rs_[0] == rmax, ix_[0], float(S)), jnp.where(rs_[1] == rmax, ix_[1], float(S)))
        idxf = jnp.min(cand, keepdims=True)

        zrow = jnp.concatenate([jnp.sum(st['z'][k], axis=0, keepdims=True) for k in range(2)], axis=1)
        zcol[...] = jnp.broadcast_to(zrow, (128, D)).T

        def q_block(b, mid=None):
            P = {}
            for n, r in enumerate(ORDER):
                if mid is not None and n == opt.get('qmid', 1): mid()
                P[r] = NT(unpack(wqtf[pl.ds(r*(dd//2), dd//2), :]), xform(r, b))
            o = [[None, None], [None, None]]
            for (i, k) in [(1, 0), (0, 1), (0, 0), (1, 1)]:
                zc = zcol[pl.ds(k*dd, dd), :]
                zc = jnp.concatenate([zc] * (tm // 128), axis=1)
                pq = phi(comb(P, GAMMA, i, k))
                t = (pq * zc).reshape(dd // DH, DH, tm)
                den = jnp.sum(t, axis=1, keepdims=True) + 1e-6
                o[k][i] = (pq.reshape(dd // DH, DH, tm) * (1.0 / den)).reshape(dd, tm)
            for r in range(R):
                of[pl.ds((b*R + r)*(dd//2), dd//2), :] = pack(_lin(ALPHA[r].T, o))

        def of1(b, r, j2):
            return of[pl.ds((b*R + r)*(dd//2) + j2*(dd//4), dd//4), :]
        def of2(sb, r, r2):
            nz = [(j2, i2) for j2 in range(2) for i2 in range(2) if ALPHA[r2].T[j2, i2]]
            if len(nz) == 1:
                (j2, i2), = nz
                return unpack(of1(2*sb + i2, r, j2))
            return unpack(ofb[pl.ds(((sb*R + r)*R + r2)*(dd//4), dd//4), :])
        def make_of2(sb, seed=None, nt=0):
            z = None
            metro = Metro(seed) if seed is not None else None
            for r in ORDER:
                RC = opt.get('of2rc', 64)
                for rc in range(256 // RC):
                    zt = metro.tick(nt) if metro is not None else None
                    q4 = [[unpack(of[pl.ds(((2*sb + i2)*R + r)*(dd//2) + j2*(dd//4) + rc*(RC//2), RC//2), :]).astype(f32) for i2 in range(2)] for j2 in range(2)]
                    if zt is not None:
                        zz = jnp.concatenate([jnp.concatenate([zt] * 2, axis=1)] * (RC // 8), axis=0)
                        q4[0][0] = q4[0][0] + zz; q4[1][1] = q4[1][1] + zz
                    for r2 in range(R):
                        if np.abs(ALPHA[r2]).sum() == 1: continue
                        v = _lin(ALPHA[r2].T, q4)
                        if opt.get('of2chain') and z is not None:
                            v = v + jnp.concatenate([jnp.concatenate([z] * 2, axis=1)] * (RC // 8), axis=0)
                        if opt.get('of2chain'): z = v[:8, :128] * 0.0
                        ofb[pl.ds(((sb*R + r)*R + r2)*(dd//4) + rc*(RC//2), RC//2), :] = pack(v)

        nq_pre = opt.get('nq_pre', 1)
        def ffn_waits(): W(cwg, 'w_wg'); W(cwu, 'w_wu')
        for b in range(nq_pre):
            if LA == 2 and b == opt.get('of2pos', 2): make_of2(0)
            q_block(b, mid=ffn_waits if (b == nq_pre - 1 and opt.get('qmid', 1) > 0) else None)

        def b_path():
            idx = jnp.clip(jnp.max(idxf).astype(i32), 0, S - 1)
            i16 = pl.multiple_of((idx // 16) * 16, 16)
            W(cwg, 'w_wg'); W(cwu, 'w_wu'); W(cwd, 'w_wd')
            _, _, d16, var16, inv16 = ln_core(x_v[pl.ds(i16, 16), :])
            xs = (d16 * inv16).astype(bf16)
            gg = rnd(NN(xs, wg_v[...]))
            uu = rnd(NN(xs, wu_v[...]))
            hh = (rnd(gg * jax.nn.sigmoid(gg)) * uu).astype(bf16)
            yy = NN(hh, wd_v[...]) * jax.nn.sigmoid(rmax)
            rowm = lax.broadcasted_iota(i32, (16, D), 0) == (idx - i16)
            st['yy'] = jnp.where(rowm, yy, 0.0); st['i16'] = i16


        CW = opt.get('cw', 512)
        def bv_stage0():
            idx = jnp.clip(jnp.max(idxf).astype(i32), 0, S - 1)
            i16 = pl.multiple_of((idx // 16) * 16, 16)
            x16 = x_v[pl.ds(i16, 16), :].astype(f32)
            mean = jnp.concatenate([st_mean[pl.ds(i16, 16), :]] * (D // 128), axis=1)
            inv = jnp.concatenate([st_inv[pl.ds(i16, 16), :]] * (D // 128), axis=1)
            xs = rnd((x16 - mean) * inv)
            rowm = lax.broadcasted_iota(i32, (16, D), 0) == (idx - i16)
            xrow = jnp.sum(jnp.where(rowm, xs, 0.0), axis=0, keepdims=True)
            xcol[...] = jnp.broadcast_to(xrow, (128, D)).T
            st['i16'] = i16; st['rowm'] = rowm
        def matvec(w_ref, col_ref, nrows, c0, cw, seg=None, z=None, metro=None, nt=0):
            acc = None
            for i in range(nrows // 8):
                if metro is not None and i % seg == 0:
                    z = metro.tick(nt)
                elif metro is None and seg and i % seg == 0 and i > 0:
                    z = gate(acc[:, :128])
                w = w_ref[pl.ds(8*i, 8), pl.ds(c0, cw)].astype(f32)
                xc = col_ref[pl.ds(8*i, 8), :]
                if cw > 128: xc = jnp.concatenate([xc] * (cw // 128), axis=1)
                t = w * xc
                if z is not None:
                    t = t + (jnp.concatenate([z] * (cw // 128), axis=1) if cw > 128 else z); z = None
                acc = t if acc is None else acc + t
            return acc
        def bv_stage1_serial(c0, c1):
            z = st.get('b1z')
            for c in range(c0, c1):
                ga = matvec(wg_v, xcol, D, c*128, 128, z=z); z = ozero(ga)
                ua = matvec(wu_v, xcol, D, c*128, 128, z=z); z = ozero(ua)
                gg = rnd(jnp.sum(ga, axis=0, keepdims=True))
                uu = rnd(jnp.sum(ua, axis=0, keepdims=True))
                hh = rnd(rnd(gg * jax.nn.sigmoid(gg)) * uu)
                hcol[pl.ds(c*128, 128), :] = jnp.broadcast_to(hh, (128, 128)).T
            st['b1z'] = z
        def bv_stage2_serial():
            z = st.get('b1z') if opt.get('b1late', 0) else None; ys = []
            for n in range(D // 128):
                ya = matvec(wd_v, hcol, F, n*128, 128, z=z); z = ozero(ya)
                ys.append(jnp.sum(ya, axis=0, keepdims=True))
            st['yacc'] = ya
            yy = jnp.concatenate(ys, axis=1) * jax.nn.sigmoid(rmax)
            st['yy'] = jnp.where(st['rowm'], yy, 0.0)
        def bv_stage1(c0, c1):
            if opt.get('serial'): return bv_stage1_serial(c0, c1)
            z = None
            m1 = Metro(xcol[pl.ds(0, 8), :]) if opt.get('nt1') else None
            for c in range(F // CW):
                ga = matvec(wg_v, xcol, D, c*CW, CW, seg=opt.get('seg1'), z=z, metro=m1, nt=opt.get('nt1', 0))
                if opt.get('chain1') == 2: z = gate(ga[:, :128])
                ua = matvec(wu_v, xcol, D, c*CW, CW, seg=opt.get('seg1'), z=z, metro=m1, nt=opt.get('nt1', 0))
                if opt.get('chain1'): z = gate(ua[:, :128])
                gg = rnd(jnp.sum(ga, axis=0, keepdims=True))
                uu = rnd(jnp.sum(ua, axis=0, keepdims=True))
                hh = rnd(rnd(gg * jax.nn.sigmoid(gg)) * uu)
                for j in range(CW // 128):
                    hcol[pl.ds(c*CW + j*128, 128), :] = jnp.broadcast_to(hh[:, j*128:(j+1)*128], (128, 128)).T
        def bv_stage2():
            if opt.get('serial'): return bv_stage2_serial()
            CN = opt.get('cn', 1024)
            m2 = Metro(xcol[pl.ds(0, 8), :]) if opt.get('nt2') else None
            ys = [jnp.sum(matvec(wd_v, hcol, F, n*CN, CN, seg=opt.get('seg2'), metro=m2, nt=opt.get('nt2', 0)), axis=0, keepdims=True) for n in range(D // CN)]
            yy = jnp.concatenate(ys, axis=1) * jax.nn.sigmoid(rmax)
            st['yy'] = jnp.where(st['rowm'], yy, 0.0)

        P = {}
        n1 = opt.get('g1', 4)
        if opt.get('bvpu'):
            bv_stage0()
            if opt.get('qmid', 1) == 0: W(cwg, 'w_wg'); W(cwu, 'w_wu')
            bv_stage1(0, 28 - opt.get('b1late', 0))
        for r in ORDER[:n1]:
            P[r] = TN(unpack(pkf[pl.ds(r*(S//4), S//4), :]), xform(r))
        if opt.get('bvpu'):
            W(cwd, 'w_wd')
            if opt.get('mv', True): W(cwv, 'w_wv'); W(cwo, 'w_wo')
            bv_stage1(28 - opt.get('b1late', 0), 28)
            bv_stage2()
        for r in ORDER[n1:]:
            P[r] = TN(unpack(pkf[pl.ds(r*(S//4), S//4), :]), xform(r))
        if opt.get('bvpu') and not opt.get('mv', True): W(cwv, 'w_wv'); W(cwo, 'w_wo')
        if opt.get('bpos') == 'trans': b_path()
        st['kvzero'] = jnp.concatenate([ozero(st['yacc'])] * 16, axis=0) if opt.get('bvpu') and opt.get('pin', True) else 0.0
        blk = lax.broadcasted_iota(i32, (128, 128), 0) // DH == lax.broadcasted_iota(i32, (128, 128), 1) // DH
        Mq = [[None, None], [None, None]]
        for k in range(2):
            Gk = [comb(P, _T(BETA), k, j) for j in range(2)]
            Ms = []
            for gi in range(dd // 128):
                g = k*(dd//128) + gi
                Gg = jnp.concatenate([Gk[j][gi*128:(gi+1)*128, :].astype(bf16) for j in range(2)], axis=1)
                kv = NN(Gg, wv_v[:, pl.ds(g*128, 128)])
                kv = jnp.where(blk, kv, st['kvzero']).astype(bf16)
                Ms.append(NN(kv, wo_v[pl.ds(g*128, 128), :]))
            if k == opt.get('seedk', 0): st['gseed'] = Ms[0][:8, :128] if opt.get('seedm', True) else Gk[0][:8, :128]
            Mk = jnp.concatenate(Ms, axis=0)
            Mq[k] = [Mk[:, :dd], Mk[:, dd:]]
        for r in range(R):
            f1 = _lin(BETA[r], Mq)
            if LA == 1:
                mf[pl.ds(r*(dd//2), dd//2), :] = pack(f1)
            else:
                q4 = [[f1[j*(dd//2):(j+1)*(dd//2), k*(dd//2):(k+1)*(dd//2)] for k in range(2)] for j in range(2)]
                for r2 in range(R):
                    mf[pl.ds((r*R + r2)*(dd//4), dd//4), :] = pack(_lin(BETA[r2], q4))

        if opt.get('bpos') == 'posttrans': b_path()
        for b in range(nq_pre, NB):
            if LA == 2 and b == opt.get('of2pos', 2): make_of2(0, seed=st['gseed'] if opt.get('nt0') is not None else None, nt=opt.get('nt0'))
            q_block(b)

        if opt.get('bpos', 'late') == 'late' and not opt.get('bvpu'): b_path()

        pend = []
        def a_piece(b, c0, nc, split_cols):
            P = {}
            for r in ORDER:
                P[r] = TN(unpack(of[pl.ds((b*R + r)*(dd//2), dd//2), pl.ds(c0*16, nc*16)]), unpack(mf[pl.ds(r*(dd//2), dd//2), :]))
            row0 = b*TM + c0*32; nrows = nc*32
            i16 = st['i16']; yy = st['yy']
            def emit(i, k):
                Aq = comb(P, GAMMA, i, k)
                for c in range(nc):
                    r0 = row0 + c*32 + i*16
                    xx = x_v[pl.ds(r0, 16), pl.ds(k*dd, dd)].astype(f32)
                    mean = jnp.concatenate([st_mean[pl.ds(r0, 16), :]] * (dd // 128), axis=1)
                    inv = jnp.concatenate([st_inv[pl.ds(r0, 16), :]] * (dd // 128), axis=1)
                    o = (Aq[c*16:(c+1)*16, :] + xx) + (xx - mean) * inv
                    out_v[pl.ds(r0, 16), pl.ds(k*dd, dd)] = o.astype(bf16)
            def patch_and_send(col0, ncol):
                off = pl.multiple_of(jnp.clip(i16 - row0, 0, nrows - 16), 16) + row0
                inb = jnp.logical_and(i16 >= row0, i16 < row0 + nrows)
                tile = out_v[pl.ds(off, 16), pl.ds(col0, ncol)].astype(f32) + jnp.where(inb, yy[:, col0:col0+ncol], 0.0)
                out_v[pl.ds(off, 16), pl.ds(col0, ncol)] = tile.astype(bf16)
                c = copy(out_v.at[pl.ds(row0, nrows), pl.ds(col0, ncol)], out_hbm.at[pl.ds(row0, nrows), pl.ds(col0, ncol)])
                c.start(); pend.append(c)
            if split_cols:
                emit(1, 0); emit(0, 1); emit(0, 0); patch_and_send(0, dd)
                emit(1, 1); patch_and_send(dd, dd)
            else:
                for (i, k) in [(1, 0), (0, 1), (0, 0), (1, 1)]: emit(i, k)
                patch_and_send(0, D)
        def a_super(sb, last, hook=None):
            i16 = st['i16']; yy = st['yy']
            Q = {}
            def send(r0, nr, col0, ncol):
                off = pl.multiple_of(jnp.clip(i16 - r0, 0, nr - 16), 16) + r0
                inb = jnp.logical_and(i16 >= r0, i16 < r0 + nr)
                tile = out_v[pl.ds(off, 16), pl.ds(col0, ncol)].astype(f32) + jnp.where(inb, yy[:, col0:col0+ncol], 0.0)
                out_v[pl.ds(off, 16), pl.ds(col0, ncol)] = tile.astype(bf16)
                c = copy(out_v.at[pl.ds(r0, nr), pl.ds(col0, ncol)], out_hbm.at[pl.ds(r0, nr), pl.ds(col0, ncol)])
                c.start(); pend.append(c)
            def emit(i2, k2, i1, k1, Qd):
                Aq = comb({ro: Qd[ro] for ro in Qd}, GAMMA, i2, k2)
                col0 = k1*dd + k2*(dd//2); b = 2*sb + i2
                for c in range(16):
                    r0 = b*TM + c*32 + i1*16
                    xx = x_v[pl.ds(r0, 16), pl.ds(col0, dd//2)].astype(f32)
                    mean = jnp.concatenate([st_mean[pl.ds(r0, 16), :]] * (dd // 256), axis=1)
                    inv = jnp.concatenate([st_inv[pl.ds(r0, 16), :]] * (dd // 256), axis=1)
                    o = (Aq[c*16:(c+1)*16, :] + xx) + (xx - mean) * inv
                    out_v[pl.ds(r0, 16), pl.ds(col0, dd//2)] = o.astype(bf16)
            QO = [(1, 0), (0, 1), (0, 0), (1, 1)]
            done = set()
            for n, ro in enumerate(ORDER):
                P2 = {ri: TN(of2(sb, ri, ro), unpack(mf[pl.ds((ri*R + ro)*(dd//4), dd//4), :])) for ri in ORDER}
                Q[ro] = {(i1, k1): comb(P2, GAMMA, i1, k1) for (i1, k1) in QO}
                if n == 0 and hook is not None: hook(Q[ro][1, 0][:8, :128])
                for (i2, k2) in QO:
                    if (i2, k2) not in done and all(rr in Q for rr in range(R) if GAMMA[rr][i2, k2]):
                        done.add((i2, k2))
                        r0 = (2*sb + i2)*TM
                        for (i1, k1) in QO:
                            emit(i2, k2, i1, k1, {rr: Q[rr][i1, k1] for rr in Q})
                            if last and (i1, k1) == (0, 0): send(r0, TM, k2*(dd//2), dd//2)
                        if last: send(r0, TM, dd + k2*(dd//2), dd//2)
                        elif k2 == (0 if i2 == 0 else 1):
                            send(r0, TM, 0, D)
        tail = opt.get('tail', 2)
        if LA == 2:
            a_super(0, False, hook=lambda seed: make_of2(1, seed=seed if opt.get('nt1') is not None else None, nt=opt.get('nt1')))
            a_super(1, True)
            tail = -1
        for b in range(NB - 1 if tail >= 0 else 0): a_piece(b, 0, 16, False)
        if tail == 0: a_piece(NB - 1, 0, 16, False)
        elif tail == 1: a_piece(NB - 1, 0, 16, True)
        elif tail == 2: a_piece(NB - 1, 0, 8, False); a_piece(NB - 1, 8, 8, True)
        elif tail == 3: a_piece(NB - 1, 0, 8, False); a_piece(NB - 1, 8, 8, False)
        for n, c in enumerate(pend): W(c, f'w_out{n}')
        assert nsem[0] <= 40
    return kernel

def build(vmem=120, flags={'XLA_TPU_EVENLY_DISTRIBUTE_CRITICAL_NODES': True}, **opt):
    kern = make_kernel(opt)
    scratch = [
        pltpu.VMEM((S, D), bf16), pltpu.VMEM((D, D), bf16), pltpu.VMEM((D, D), bf16), pltpu.VMEM((D, D), bf16), pltpu.VMEM((D, D), bf16),
        pltpu.VMEM((8, 128), bf16), pltpu.VMEM((D, F), bf16), pltpu.VMEM((D, F), bf16), pltpu.VMEM((F, D), bf16),
        pltpu.VMEM((S, 128), f32), pltpu.VMEM((S, 128), f32),
        pltpu.VMEM((R * S // 4, dd), u32), pltpu.VMEM((R * S // 4, dd), u32),
        pltpu.VMEM((R * dd // 2, dd), u32), pltpu.VMEM((R * dd // 2, dd), u32),
        pltpu.VMEM((NB * R * dd // 2, tm), u32),
        pltpu.VMEM((R * dd // 2, dd), u32) if opt.get('LA', 1) == 1 else pltpu.VMEM((R * R * dd // 4, dd // 2), u32),
        pltpu.VMEM((D, 128), f32), pltpu.VMEM((S, D), bf16), pltpu.VMEM((D, 128), f32), pltpu.VMEM((F, 128), f32), pltpu.VMEM((24, 128), bf16), pltpu.VMEM((2 * R * R * dd // 4, tm), u32) if opt.get('LA', 1) == 2 else pltpu.VMEM((8, 128), u32),
        pltpu.SemaphoreType.DMA((40,)),
    ]
    any_spec = pl.BlockSpec(memory_space=pl.ANY)
    @jax.jit
    def fn(A_x, A_wqkv, A_wo, B_x, B_w_r, B_w_gate, B_w_up, B_w_down):
        out = pl.pallas_call(
            kern,
            out_shape=jax.ShapeDtypeStruct((S, D), bf16),
            in_specs=[any_spec] * 7, out_specs=any_spec,
            scratch_shapes=scratch,
            compiler_params=pltpu.CompilerParams(vmem_limit_bytes=vmem * 1024 * 1024, flags=flags),
            name="la_moe_k5",
        )(A_x.reshape(S, D), A_wqkv, A_wo, B_w_r.reshape(8, 128), B_w_gate, B_w_up, B_w_down)
        return out.reshape(1, S, D)
    return fn


_impl = build(bvpu=True,nq_pre=3,serial=True,g1=5,qmid=0,nx0=2,LA=2,of2pos=3,nt0=3,nt1=3,seedk=1)


@jax.jit
def pallas_parallel_sum__linear_attn_block__moe_arch_mod__prompt_kernel(
    A_x, A_wqkv, A_wo, B_x, B_w_r, B_w_gate, B_w_up, B_w_down):
    return _impl(A_x, A_wqkv, A_wo, B_x, B_w_r, B_w_gate, B_w_up, B_w_down)
```

```python
import numpy as np
import jax
import jax.numpy as jnp
from jax import lax
import jax.experimental.pallas as pl
import jax.experimental.pallas.tpu as pltpu

f32, bf16, u32, i32 = jnp.float32, jnp.bfloat16, jnp.uint32, jnp.int32

S, D, DH, F = 2048, 1024, 32, 3584
TM = 512
NB = S // TM
tm = TM // 2
dd = D // 2
R = 7


def _table(*terms):
    m = np.zeros((2, 2), int)
    for (sign, i, j) in terms:
        m[i, j] = sign
    return m


ALPHA = [_table((1, 0, 0), (1, 1, 1)), _table((1, 1, 0), (1, 1, 1)), _table((1, 0, 0)), _table((1, 1, 1)),
         _table((1, 0, 0), (1, 0, 1)), _table((1, 1, 0), (-1, 0, 0)), _table((1, 0, 1), (-1, 1, 1))]
BETA = [_table((1, 0, 0), (1, 1, 1)), _table((1, 0, 0)), _table((1, 0, 1), (-1, 1, 1)), _table((1, 1, 0), (-1, 0, 0)),
        _table((1, 1, 1)), _table((1, 0, 0), (1, 0, 1)), _table((1, 1, 0), (1, 1, 1))]
GAMMA = [_table((1, 0, 0), (1, 1, 1)), _table((1, 1, 0), (-1, 1, 1)), _table((1, 0, 1), (1, 1, 1)),
         _table((1, 0, 0), (1, 1, 0)), _table((-1, 0, 0), (1, 0, 1)), _table((1, 1, 1)), _table((1, 0, 0))]
BETA_T = [m.T for m in BETA]

ORDER_A = [1, 3, 4, 2, 0, 6, 5]
ORDER_B = [0, 1, 3, 6, 4, 2, 5]


def _quadrants(order):
    out = []
    for n in range(1, R + 1):
        have = set(order[:n])
        for q in [(1, 0), (0, 1), (0, 0), (1, 1)]:
            if q not in out and all(r in have for r in range(R) if GAMMA[r][q]):
                out.append(q)
    return out


def _signed_sum(pos, neg):
    acc = pos[0]
    for t in pos[1:]:
        acc = acc + t
    for t in neg:
        acc = acc - t
    return acc


def form(c, blocks):
    idx = [(i, j) for i in range(2) for j in range(2)]
    return _signed_sum([blocks[i][j] for i, j in idx if c[i, j] > 0], [blocks[i][j] for i, j in idx if c[i, j] < 0])


def combine(P, coef, i, k):
    return _signed_sum([P[r] for r in range(R) if coef[r][i, k] > 0], [P[r] for r in range(R) if coef[r][i, k] < 0])


def rnd(x):
    return x.astype(bf16).astype(f32)


def phi(t):
    return jnp.where(t > 0, t + 1.0, jnp.exp(t)) + 1e-6


def NN(a, b):
    return jnp.dot(a, b, preferred_element_type=f32)


def NT(a, b):
    return lax.dot_general(a, b, (((1,), (1,)), ((), ())), preferred_element_type=f32)


def TN(a, b):
    return lax.dot_general(a, b, (((0,), (0,)), ((), ())), preferred_element_type=f32)


def pack(x):
    return pltpu.bitcast(x.astype(bf16), u32)


def unpack(x):
    return pltpu.bitcast(x, bf16)


def after(a):
    u = pltpu.bitcast(a, i32)
    return jnp.where(jnp.minimum(u, 5) <= jnp.maximum(u, 3), 0.0, a)


class Pacer:
    def __init__(self, start):
        u = pltpu.bitcast(start, i32)
        self.t = jnp.where(jnp.minimum(u, 5) <= jnp.maximum(u, 3), 1.0, start)

    def tick(self, n):
        for _ in range(n):
            self.t = jnp.broadcast_to(jnp.sum(self.t, axis=-1, keepdims=True), (8, 128)) * (1.0 / 128)
        return after(self.t)


def _kernel(x_hbm, wqkv_hbm, wo_hbm, wr_hbm, wg_hbm, wu_hbm, wd_hbm, out_hbm,
            x_v, wq_v, wk_v, wv_v, wo_v, wr_v, wg_v, wu_v, wd_v,
            st_mean, st_inv, xf, pkf, wkf, wqtf, of, mf, zcol, out_v, xcol, hcol, of2, sems):
    nsem = [0]

    def copy(src, dst):
        nsem[0] += 1
        return pltpu.make_async_copy(src, dst, sems.at[nsem[0] - 1])

    cx0 = [copy(x_hbm.at[pl.ds(i * tm, tm), :], x_v.at[pl.ds(i * tm, tm), :]) for i in range(2)]
    cx = [None] + [copy(x_hbm.at[pl.ds(b * TM, TM), :], x_v.at[pl.ds(b * TM, TM), :]) for b in range(1, NB)]
    cwk = [copy(wqkv_hbm.at[pl.ds(j * dd, dd), pl.ds(D, D)], wk_v.at[pl.ds(j * dd, dd), :]) for j in range(2)]
    cwq = copy(wqkv_hbm.at[:, pl.ds(0, D)], wq_v)
    cwv = copy(wqkv_hbm.at[:, pl.ds(2 * D, D)], wv_v)
    cwo = copy(wo_hbm, wo_v)
    cwr = copy(wr_hbm, wr_v)
    cwg, cwu, cwd = copy(wg_hbm, wg_v), copy(wu_hbm, wu_v), copy(wd_hbm, wd_v)
    for c in [cwr] + cx0 + cwk + [cx[1], cx[2], cx[3], cwq, cwg, cwu, cwd, cwv, cwo]:
        c.start()

    lane = lax.broadcasted_iota(i32, (8, 128), 1)
    cvar = [jnp.zeros((8, 128), f32) for _ in range(2)]
    cdot = [jnp.zeros((8, 128), f32) for _ in range(2)]
    zsum = [None, None]

    def ln_chunk(b, c, wr):
        r0 = b * TM + c * 32
        xv = x_v[pl.ds(r0, 32), :].astype(f32)
        mean = jnp.sum(xv, axis=-1, keepdims=True) * (1.0 / D)
        d = xv - mean
        var = jnp.sum(d * d, axis=-1, keepdims=True) * (1.0 / D)
        inv = lax.rsqrt(var + 1e-5)
        xn = d * inv
        st_mean[pl.ds(r0, 32), :] = jnp.broadcast_to(mean, (32, 128))
        st_inv[pl.ds(r0, 32), :] = jnp.broadcast_to(inv, (32, 128))
        X = [[xn[:16, :dd], xn[:16, dd:]], [xn[16:, :dd], xn[16:, dd:]]]
        for r in range(R):
            xf[pl.ds(r * (S // 4) + b * (tm // 2) + c * 8, 8), :] = pack(form(ALPHA[r], X))
        acc = None
        for j in range(D // 128):
            t = d[:, j * 128:(j + 1) * 128] * wr[j:j + 1, :]
            acc = t if acc is None else acc + t
        dot = jnp.sum(acc, axis=-1, keepdims=True)
        for g in range(4):
            gi = r0 // 8 + g
            sel = lane == (gi % 128)
            cvar[gi // 128] = jnp.where(sel, var[g * 8:(g + 1) * 8, :], cvar[gi // 128])
            cdot[gi // 128] = jnp.where(sel, dot[g * 8:(g + 1) * 8, :], cdot[gi // 128])

    def xform(r, b=None):
        if b is None:
            return unpack(xf[pl.ds(r * (S // 4), S // 4), :])
        return unpack(xf[pl.ds(r * (S // 4) + b * (tm // 2), tm // 2), :])

    def wk_form(r):
        if r == 1:
            return wk_v[pl.ds(0, dd), pl.ds(0, dd)]
        if r == 4:
            return wk_v[pl.ds(dd, dd), pl.ds(dd, dd)]
        return unpack(wkf[pl.ds(r * (dd // 2), dd // 2), :])

    def weight_forms(src, dst, rs, transpose=False):
        for rc in range(dd // 128):
            need = sorted({(j, k) for r in rs for j in range(2) for k in range(2) if BETA[r][j, k]})
            blocks = [[None, None], [None, None]]
            for (j, k) in need:
                blocks[j][k] = src[pl.ds(j * dd + rc * 128, 128), pl.ds(k * dd, dd)].astype(f32)
            for r in rs:
                v = form(BETA[r], blocks)
                if transpose:
                    dst[pl.ds(r * (dd // 2), dd // 2), pl.ds(rc * 128, 128)] = pltpu.bitcast(v.astype(bf16).T, u32)
                else:
                    dst[pl.ds(r * (dd // 2) + rc * 64, 64), :] = pack(v)

    def k_products(b, rs, P):
        for r in rs:
            P[r] = NN(xform(r, b), wk_form(r))

    def k_finish(b, P, quadrants):
        pk = [[None, None], [None, None]]
        for (i, k) in quadrants:
            pk[i][k] = phi(combine(P, GAMMA, i, k))
            zz = jnp.sum(pk[i][k].reshape(tm // 8, 8, dd), axis=0)
            zsum[k] = zz if zsum[k] is None else zsum[k] + zz
        for r in range(R):
            pkf[pl.ds(r * (S // 4) + b * (tm // 2), tm // 2), :] = pack(form(GAMMA[r], pk))

    def k_block(b):
        P = {}
        k_products(b, ORDER_B, P)
        k_finish(b, P, _quadrants(ORDER_B))

    cwr.wait()
    wr = wr_v[...].astype(f32)
    for i in range(2):
        cx0[i].wait()
        for c in range(8 * i, 8 * i + 8):
            ln_chunk(0, c, wr)
    P = {}
    cwk[0].wait()
    weight_forms(wk_v, wkf, [5])
    k_products(0, [1, 5], P)
    cwk[1].wait()
    weight_forms(wk_v, wkf, [2, 3, 0, 6])
    k_products(0, [4, 2], P)
    cx[1].wait()
    for c in range(16):
        ln_chunk(1, c, wr)
    k_products(0, [3, 0, 6], P)
    k_finish(0, P, [(0, 1), (1, 0), (1, 1), (0, 0)])
    for b in (1, 2):
        cx[b + 1].wait()
        for c in range(16):
            ln_chunk(b + 1, c, wr)
        k_block(b)
    cwq.wait()
    weight_forms(wq_v, wqtf, range(R), transpose=True)
    k_block(3)

    sub = lax.broadcasted_iota(i32, (8, 128), 0)
    score, token = [], []
    for h in range(2):
        s_ref = rnd(jnp.sqrt(rnd(rnd(cvar[h]) + rnd(jnp.float32(1e-5)))))
        score.append(rnd(cdot[h] * (1.0 / s_ref)))
        token.append(((lane + h * 128) * 8 + sub).astype(f32))
    rmax = jnp.max(jnp.maximum(score[0], score[1]), keepdims=True)
    cand = jnp.minimum(jnp.where(score[0] == rmax, token[0], float(S)), jnp.where(score[1] == rmax, token[1], float(S)))
    idxf = jnp.min(cand, keepdims=True)

    zrow = jnp.concatenate([jnp.sum(zsum[k], axis=0, keepdims=True) for k in range(2)], axis=1)
    zcol[...] = jnp.broadcast_to(zrow, (128, D)).T

    def q_block(b):
        P = {}
        for r in ORDER_B:
            P[r] = NT(unpack(wqtf[pl.ds(r * (dd // 2), dd // 2), :]), xform(r, b))
        o = [[None, None], [None, None]]
        for (i, k) in _quadrants(ORDER_B):
            zc = zcol[pl.ds(k * dd, dd), :]
            zc = jnp.concatenate([zc] * (tm // 128), axis=1)
            pq = phi(combine(P, GAMMA, i, k))
            t = (pq * zc).reshape(dd // DH, DH, tm)
            den = jnp.sum(t, axis=1, keepdims=True) + 1e-6
            o[k][i] = (pq.reshape(dd // DH, DH, tm) * (1.0 / den)).reshape(dd, tm)
        for r in range(R):
            of[pl.ds((b * R + r) * (dd // 2), dd // 2), :] = pack(form(ALPHA[r].T, o))

    def o_form2(sb, r, r2):
        nz = [(j2, i2) for j2 in range(2) for i2 in range(2) if ALPHA[r2].T[j2, i2]]
        if len(nz) == 1:
            (j2, i2), = nz
            return unpack(of[pl.ds(((2 * sb + i2) * R + r) * (dd // 2) + j2 * (dd // 4), dd // 4), :])
        return unpack(of2[pl.ds(((sb * R + r) * R + r2) * (dd // 4), dd // 4), :])

    def make_o_form2(sb, start):
        pacer = Pacer(start)
        for r in ORDER_A:
            for rc in range(4):
                z = pacer.tick(3)
                q4 = [[unpack(of[pl.ds(((2 * sb + i2) * R + r) * (dd // 2) + j2 * (dd // 4) + rc * 32, 32), :]).astype(f32)
                       for i2 in range(2)] for j2 in range(2)]
                zz = jnp.concatenate([jnp.concatenate([z] * 2, axis=1)] * 8, axis=0)
                q4[0][0] = q4[0][0] + zz
                q4[1][1] = q4[1][1] + zz
                for r2 in range(R):
                    if np.abs(ALPHA[r2]).sum() > 1:
                        of2[pl.ds(((sb * R + r) * R + r2) * (dd // 4) + rc * 32, 32), :] = pack(form(ALPHA[r2].T, q4))

    for b in range(NB - 1):
        q_block(b)

    idx = jnp.clip(jnp.max(idxf).astype(i32), 0, S - 1)
    i16 = pl.multiple_of((idx // 16) * 16, 16)
    x16 = x_v[pl.ds(i16, 16), :].astype(f32)
    mean16 = jnp.concatenate([st_mean[pl.ds(i16, 16), :]] * (D // 128), axis=1)
    inv16 = jnp.concatenate([st_inv[pl.ds(i16, 16), :]] * (D // 128), axis=1)
    xs = rnd((x16 - mean16) * inv16)
    rowm = lax.broadcasted_iota(i32, (16, D), 0) == (idx - i16)
    xrow = jnp.sum(jnp.where(rowm, xs, 0.0), axis=0, keepdims=True)
    xcol[...] = jnp.broadcast_to(xrow, (128, D)).T

    def matvec(w_ref, col_ref, nrows, c0, z):
        acc = None
        for i in range(nrows // 8):
            t = w_ref[pl.ds(8 * i, 8), pl.ds(c0, 128)].astype(f32) * col_ref[pl.ds(8 * i, 8), :]
            if i == 0 and z is not None:
                t = t + z
            acc = t if acc is None else acc + t
        return acc

    def pk_form(r):
        return unpack(pkf[pl.ds(r * (S // 4), S // 4), :])

    P = {}
    lhs = pk_form(ORDER_A[0]).T
    cwg.wait()
    cwu.wait()
    z = None
    for c in range(F // 128):
        ga = matvec(wg_v, xcol, D, c * 128, z)
        z = after(ga)
        ua = matvec(wu_v, xcol, D, c * 128, z)
        z = after(ua)
        gg = rnd(jnp.sum(ga, axis=0, keepdims=True))
        uu = rnd(jnp.sum(ua, axis=0, keepdims=True))
        hh = rnd(rnd(gg * jax.nn.sigmoid(gg)) * uu)
        hcol[pl.ds(c * 128, 128), :] = jnp.broadcast_to(hh, (128, 128)).T
    P[ORDER_A[0]] = NN(lhs, xform(ORDER_A[0]))
    for r in ORDER_A[1:4]:
        P[r] = TN(pk_form(r), xform(r))
    lhs = pk_form(ORDER_A[4]).T
    cwd.wait()
    cwv.wait()
    cwo.wait()
    z, ys = None, []
    for n in range(D // 128):
        ya = matvec(wd_v, hcol, F, n * 128, z)
        z = after(ya)
        ys.append(jnp.sum(ya, axis=0, keepdims=True))
    yy = jnp.where(rowm, jnp.concatenate(ys, axis=1) * jax.nn.sigmoid(rmax), 0.0)
    P[ORDER_A[4]] = NN(lhs, xform(ORDER_A[4]))
    for r in ORDER_A[5:]:
        P[r] = TN(pk_form(r), xform(r))

    zero = jnp.concatenate([after(ya)] * 16, axis=0)
    blk = lax.broadcasted_iota(i32, (128, 128), 0) // DH == lax.broadcasted_iota(i32, (128, 128), 1) // DH
    Mq = [None, None]
    for k in range(2):
        Gk = [combine(P, BETA_T, k, j) for j in range(2)]
        Ms = []
        for gi in range(dd // 128):
            g = k * (dd // 128) + gi
            Gg = jnp.concatenate([Gk[j][gi * 128:(gi + 1) * 128, :].astype(bf16) for j in range(2)], axis=1)
            kv = NN(Gg, wv_v[:, pl.ds(g * 128, 128)])
            kv = jnp.where(blk, kv, zero).astype(bf16)
            Ms.append(NN(kv, wo_v[pl.ds(g * 128, 128), :]))
        m_start = Ms[0][:8, :128]
        Mk = jnp.concatenate(Ms, axis=0)
        Mq[k] = [Mk[:, :dd], Mk[:, dd:]]
    for r in range(R):
        f1 = form(BETA[r], Mq)
        q4 = [[f1[j * (dd // 2):(j + 1) * (dd // 2), k * (dd // 2):(k + 1) * (dd // 2)] for k in range(2)] for j in range(2)]
        for r2 in range(R):
            mf[pl.ds((r * R + r2) * (dd // 4), dd // 4), :] = pack(form(BETA[r2], q4))

    make_o_form2(0, m_start)
    q_block(NB - 1)

    pending = []

    def send(r0, col0, ncol):
        off = pl.multiple_of(jnp.clip(i16 - r0, 0, TM - 16), 16) + r0
        inside = jnp.logical_and(i16 >= r0, i16 < r0 + TM)
        tile = out_v[pl.ds(off, 16), pl.ds(col0, ncol)].astype(f32) + jnp.where(inside, yy[:, col0:col0 + ncol], 0.0)
        out_v[pl.ds(off, 16), pl.ds(col0, ncol)] = tile.astype(bf16)
        c = copy(out_v.at[pl.ds(r0, TM), pl.ds(col0, ncol)], out_hbm.at[pl.ds(r0, TM), pl.ds(col0, ncol)])
        c.start()
        pending.append(c)

    def emit(b, i1, col0, Aq):
        for c in range(16):
            r0 = b * TM + c * 32 + i1 * 16
            xx = x_v[pl.ds(r0, 16), pl.ds(col0, dd // 2)].astype(f32)
            mean = jnp.concatenate([st_mean[pl.ds(r0, 16), :]] * (dd // 256), axis=1)
            inv = jnp.concatenate([st_inv[pl.ds(r0, 16), :]] * (dd // 256), axis=1)
            o = (Aq[c * 16:(c + 1) * 16, :] + xx) + (xx - mean) * inv
            out_v[pl.ds(r0, 16), pl.ds(col0, dd // 2)] = o.astype(bf16)

    for sb in range(NB // 2):
        last = sb == NB // 2 - 1
        Q, done = {}, set()
        for n, ro in enumerate(ORDER_B):
            P2 = {ri: TN(o_form2(sb, ri, ro), unpack(mf[pl.ds((ri * R + ro) * (dd // 4), dd // 4), :])) for ri in ORDER_A}
            Q[ro] = {q: combine(P2, GAMMA, *q) for q in [(1, 0), (0, 1), (0, 0), (1, 1)]}
            if n == 0 and not last:
                make_o_form2(sb + 1, Q[ro][1, 0][:8, :128])
            for (i2, k2) in [(1, 0), (0, 1), (0, 0), (1, 1)]:
                if (i2, k2) in done or not all(r in Q for r in range(R) if GAMMA[r][i2, k2]):
                    continue
                done.add((i2, k2))
                b = 2 * sb + i2
                fin = set()
                for (i1, k1) in _quadrants(ORDER_A):
                    emit(b, i1, k1 * dd + k2 * (dd // 2), combine({r: Q[r][i1, k1] for r in Q}, GAMMA, i2, k2))
                    fin.add((i1, k1))
                    if last and (1 - i1, k1) in fin:
                        send(b * TM, k1 * dd + k2 * (dd // 2), dd // 2)
                if not last and (i2, 1 - k2) in done:
                    send(b * TM, 0, D)
    for c in pending:
        c.wait()


@jax.jit
def pallas_parallel_sum__linear_attn_block__moe_arch_mod__prompt_kernel(
    A_x: jax.Array,
    A_wqkv: jax.Array,
    A_wo: jax.Array,
    B_x: jax.Array,
    B_w_r: jax.Array,
    B_w_gate: jax.Array,
    B_w_up: jax.Array,
    B_w_down: jax.Array,
):
    scratch = [
        pltpu.VMEM((S, D), bf16),
        pltpu.VMEM((D, D), bf16), pltpu.VMEM((D, D), bf16), pltpu.VMEM((D, D), bf16), pltpu.VMEM((D, D), bf16),
        pltpu.VMEM((8, 128), bf16),
        pltpu.VMEM((D, F), bf16), pltpu.VMEM((D, F), bf16), pltpu.VMEM((F, D), bf16),
        pltpu.VMEM((S, 128), f32), pltpu.VMEM((S, 128), f32),
        pltpu.VMEM((R * S // 4, dd), u32), pltpu.VMEM((R * S // 4, dd), u32),
        pltpu.VMEM((R * dd // 2, dd), u32), pltpu.VMEM((R * dd // 2, dd), u32),
        pltpu.VMEM((NB * R * dd // 2, tm), u32),
        pltpu.VMEM((R * R * dd // 4, dd // 2), u32),
        pltpu.VMEM((D, 128), f32),
        pltpu.VMEM((S, D), bf16),
        pltpu.VMEM((D, 128), f32), pltpu.VMEM((F, 128), f32),
        pltpu.VMEM((2 * R * R * dd // 4, tm), u32),
        pltpu.SemaphoreType.DMA((24,)),
    ]
    any_spec = pl.BlockSpec(memory_space=pl.ANY)
    out = pl.pallas_call(
        _kernel,
        out_shape=jax.ShapeDtypeStruct((S, D), bf16),
        in_specs=[any_spec] * 7,
        out_specs=any_spec,
        scratch_shapes=scratch,
        compiler_params=pltpu.CompilerParams(
            vmem_limit_bytes=120 * 1024 * 1024,
            flags={"XLA_TPU_EVENLY_DISTRIBUTE_CRITICAL_NODES": True}),
    )(A_x.reshape(S, D), A_wqkv, A_wo, B_w_r.reshape(8, 128), B_w_gate, B_w_up, B_w_down)
    return out.reshape(1, S, D)
```

```python
import numpy as np
import jax
import jax.numpy as jnp
from jax import lax
import jax.experimental.pallas as pl
import jax.experimental.pallas.tpu as pltpu

f32, bf16, u32, i32 = jnp.float32, jnp.bfloat16, jnp.uint32, jnp.int32

S, D, DH, F = 2048, 1024, 32, 3584
TM = 512
NB = S // TM
tm = TM // 2
dd = D // 2
R = 7


def _table(*terms):
    m = np.zeros((2, 2), int)
    for (sign, i, j) in terms:
        m[i, j] = sign
    return m


ALPHA = [_table((1, 0, 0), (1, 1, 1)), _table((1, 1, 0), (1, 1, 1)), _table((1, 0, 0)), _table((1, 1, 1)),
         _table((1, 0, 0), (1, 0, 1)), _table((1, 1, 0), (-1, 0, 0)), _table((1, 0, 1), (-1, 1, 1))]
BETA = [_table((1, 0, 0), (1, 1, 1)), _table((1, 0, 0)), _table((1, 0, 1), (-1, 1, 1)), _table((1, 1, 0), (-1, 0, 0)),
        _table((1, 1, 1)), _table((1, 0, 0), (1, 0, 1)), _table((1, 1, 0), (1, 1, 1))]
GAMMA = [_table((1, 0, 0), (1, 1, 1)), _table((1, 1, 0), (-1, 1, 1)), _table((1, 0, 1), (1, 1, 1)),
         _table((1, 0, 0), (1, 1, 0)), _table((-1, 0, 0), (1, 0, 1)), _table((1, 1, 1)), _table((1, 0, 0))]
BETA_T = [m.T for m in BETA]

ORDER_A = [1, 3, 4, 2, 0, 6, 5]
ORDER_B = [0, 1, 3, 6, 4, 2, 5]


def _quadrants(order):
    out = []
    for n in range(1, R + 1):
        have = set(order[:n])
        for q in [(1, 0), (0, 1), (0, 0), (1, 1)]:
            if q not in out and all(r in have for r in range(R) if GAMMA[r][q]):
                out.append(q)
    return out


def _signed_sum(pos, neg):
    acc = pos[0]
    for t in pos[1:]:
        acc = acc + t
    for t in neg:
        acc = acc - t
    return acc


def form(c, blocks):
    idx = [(i, j) for i in range(2) for j in range(2)]
    return _signed_sum([blocks[i][j] for i, j in idx if c[i, j] > 0], [blocks[i][j] for i, j in idx if c[i, j] < 0])


def combine(P, coef, i, k):
    return _signed_sum([P[r] for r in range(R) if coef[r][i, k] > 0], [P[r] for r in range(R) if coef[r][i, k] < 0])


def rnd(x):
    return x.astype(bf16).astype(f32)


def phi(t):
    return jnp.where(t > 0, t + 1.0, jnp.exp(t)) + 1e-6


def NN(a, b):
    return jnp.dot(a, b, preferred_element_type=f32)


def NT(a, b):
    return lax.dot_general(a, b, (((1,), (1,)), ((), ())), preferred_element_type=f32)


def TN(a, b):
    return lax.dot_general(a, b, (((0,), (0,)), ((), ())), preferred_element_type=f32)


def pack(x):
    return pltpu.bitcast(x.astype(bf16), u32)


def unpack(x):
    return pltpu.bitcast(x, bf16)


def after(a):
    u = pltpu.bitcast(a, i32)
    return jnp.where(jnp.minimum(u, 5) <= jnp.maximum(u, 3), 0.0, a)


class Pacer:
    def __init__(self, start):
        u = pltpu.bitcast(start, i32)
        self.t = jnp.where(jnp.minimum(u, 5) <= jnp.maximum(u, 3), 1.0, start)

    def tick(self, n):
        for _ in range(n):
            self.t = jnp.broadcast_to(jnp.sum(self.t, axis=-1, keepdims=True), (8, 128)) * (1.0 / 128)
        return after(self.t)


def _kernel(x_hbm, wqkv_hbm, wo_hbm, wr_hbm, wg_hbm, wu_hbm, wd_hbm, out_hbm,
            x_v, wq_v, wk_v, wv_v, wo_v, wr_v, wg_v, wu_v, wd_v,
            st_mean, st_inv, xf, pkf, wkf, wqtf, of, mf, zcol, out_v, xcol, hcol, of2, sems):
    nsem = [0]

    def copy(src, dst):
        nsem[0] += 1
        return pltpu.make_async_copy(src, dst, sems.at[nsem[0] - 1])

    cx0 = [copy(x_hbm.at[pl.ds(i * tm, tm), :], x_v.at[pl.ds(i * tm, tm), :]) for i in range(2)]
    cx1 = [copy(x_hbm.at[pl.ds(TM + i * tm, tm), :], x_v.at[pl.ds(TM + i * tm, tm), :]) for i in range(2)]
    cx = [None, None] + [copy(x_hbm.at[pl.ds(b * TM, TM), :], x_v.at[pl.ds(b * TM, TM), :]) for b in range(2, NB)]
    cwk = [copy(wqkv_hbm.at[pl.ds(j * dd, dd), pl.ds(D, D)], wk_v.at[pl.ds(j * dd, dd), :]) for j in range(2)]
    cwq = copy(wqkv_hbm.at[:, pl.ds(0, D)], wq_v)
    cwv = copy(wqkv_hbm.at[:, pl.ds(2 * D, D)], wv_v)
    cwo = copy(wo_hbm, wo_v)
    cwr = copy(wr_hbm, wr_v)
    cwg, cwu, cwd = copy(wg_hbm, wg_v), copy(wu_hbm, wu_v), copy(wd_hbm, wd_v)
    for c in [cwr] + cx0 + cwk + cx1 + [cx[2], cx[3], cwq, cwg, cwu, cwd, cwv, cwo]:
        c.start()

    lane = lax.broadcasted_iota(i32, (8, 128), 1)
    cvar = [jnp.zeros((8, 128), f32) for _ in range(2)]
    cdot = [jnp.zeros((8, 128), f32) for _ in range(2)]
    zsum = [None, None]

    def ln_chunk(b, c, wr):
        r0 = b * TM + c * 32
        xv = x_v[pl.ds(r0, 32), :].astype(f32)
        mean = jnp.sum(xv, axis=-1, keepdims=True) * (1.0 / D)
        d = xv - mean
        var = jnp.sum(d * d, axis=-1, keepdims=True) * (1.0 / D)
        inv = lax.rsqrt(var + 1e-5)
        xn = d * inv
        st_mean[pl.ds(r0, 32), :] = jnp.broadcast_to(mean, (32, 128))
        st_inv[pl.ds(r0, 32), :] = jnp.broadcast_to(inv, (32, 128))
        X = [[xn[:16, :dd], xn[:16, dd:]], [xn[16:, :dd], xn[16:, dd:]]]
        for r in range(R):
            xf[pl.ds(r * (S // 4) + b * (tm // 2) + c * 8, 8), :] = pack(form(ALPHA[r], X))
        acc = None
        for j in range(D // 128):
            t = d[:, j * 128:(j + 1) * 128] * wr[j:j + 1, :]
            acc = t if acc is None else acc + t
        dot = jnp.sum(acc, axis=-1, keepdims=True)
        for g in range(4):
            gi = r0 // 8 + g
            sel = lane == (gi % 128)
            cvar[gi // 128] = jnp.where(sel, var[g * 8:(g + 1) * 8, :], cvar[gi // 128])
            cdot[gi // 128] = jnp.where(sel, dot[g * 8:(g + 1) * 8, :], cdot[gi // 128])

    def xform(r, b=None):
        if b is None:
            return unpack(xf[pl.ds(r * (S // 4), S // 4), :])
        return unpack(xf[pl.ds(r * (S // 4) + b * (tm // 2), tm // 2), :])

    def wk_form(r):
        if r == 1:
            return wk_v[pl.ds(0, dd), pl.ds(0, dd)]
        if r == 4:
            return wk_v[pl.ds(dd, dd), pl.ds(dd, dd)]
        return unpack(wkf[pl.ds(r * (dd // 2), dd // 2), :])

    def weight_forms(src, dst, rs, transpose=False):
        for rc in range(dd // 128):
            need = sorted({(j, k) for r in rs for j in range(2) for k in range(2) if BETA[r][j, k]})
            blocks = [[None, None], [None, None]]
            for (j, k) in need:
                blocks[j][k] = src[pl.ds(j * dd + rc * 128, 128), pl.ds(k * dd, dd)].astype(f32)
            for r in rs:
                v = form(BETA[r], blocks)
                if transpose:
                    dst[pl.ds(r * (dd // 2), dd // 2), pl.ds(rc * 128, 128)] = pltpu.bitcast(v.astype(bf16).T, u32)
                else:
                    dst[pl.ds(r * (dd // 2) + rc * 64, 64), :] = pack(v)

    def k_products(b, rs, P):
        for r in rs:
            P[r] = NN(xform(r, b), wk_form(r))

    def k_finish(b, P, quadrants):
        pk = [[None, None], [None, None]]
        for (i, k) in quadrants:
            pk[i][k] = phi(combine(P, GAMMA, i, k))
            zz = jnp.sum(pk[i][k].reshape(tm // 8, 8, dd), axis=0)
            zsum[k] = zz if zsum[k] is None else zsum[k] + zz
        for r in range(R):
            pkf[pl.ds(r * (S // 4) + b * (tm // 2), tm // 2), :] = pack(form(GAMMA[r], pk))

    def k_half(b, h):
        hm = tm // 2
        P = {}
        for r in ORDER_B:
            P[r] = NN(unpack(xf[pl.ds(r * (S // 4) + b * (tm // 2) + h * (hm // 2), hm // 2), :]), wk_form(r))
        pk = [[None, None], [None, None]]
        for (i, k) in _quadrants(ORDER_B):
            pk[i][k] = phi(combine(P, GAMMA, i, k))
            zz = jnp.sum(pk[i][k].reshape(hm // 8, 8, dd), axis=0)
            zsum[k] = zz if zsum[k] is None else zsum[k] + zz
        for r in range(R):
            pkf[pl.ds(r * (S // 4) + b * (tm // 2) + h * (hm // 2), hm // 2), :] = pack(form(GAMMA[r], pk))

    def k_block(b):
        P = {}
        k_products(b, ORDER_B, P)
        k_finish(b, P, _quadrants(ORDER_B))

    cwr.wait()
    wr = wr_v[...].astype(f32)
    for i in range(2):
        cx0[i].wait()
        for c in range(8 * i, 8 * i + 8):
            ln_chunk(0, c, wr)
    P = {}
    cwk[0].wait()
    weight_forms(wk_v, wkf, [5])
    k_products(0, [1, 5], P)
    cwk[1].wait()
    weight_forms(wk_v, wkf, [2, 3, 0, 6])
    k_products(0, [4, 2], P)
    cx1[0].wait()
    for c in range(8):
        ln_chunk(1, c, wr)
    k_products(0, [3, 0, 6], P)
    k_finish(0, P, [(0, 1), (1, 0), (1, 1), (0, 0)])
    cx1[1].wait()
    cx[2].wait()
    for c in range(8, 16):
        ln_chunk(1, c, wr)
    k_half(1, 0)
    for c in range(16):
        ln_chunk(2, c, wr)
    k_half(1, 1)
    cx[3].wait()
    for c in range(16):
        ln_chunk(3, c, wr)
    k_block(2)
    cwq.wait()
    weight_forms(wq_v, wqtf, range(R), transpose=True)
    k_block(3)

    sub = lax.broadcasted_iota(i32, (8, 128), 0)
    score, token = [], []
    for h in range(2):
        s_ref = rnd(jnp.sqrt(rnd(rnd(cvar[h]) + rnd(jnp.float32(1e-5)))))
        score.append(rnd(cdot[h] * (1.0 / s_ref)))
        token.append(((lane + h * 128) * 8 + sub).astype(f32))
    rmax = jnp.max(jnp.maximum(score[0], score[1]), keepdims=True)
    cand = jnp.minimum(jnp.where(score[0] == rmax, token[0], float(S)), jnp.where(score[1] == rmax, token[1], float(S)))
    idxf = jnp.min(cand, keepdims=True)

    zrow = jnp.concatenate([jnp.sum(zsum[k], axis=0, keepdims=True) for k in range(2)], axis=1)
    zcol[...] = jnp.broadcast_to(zrow, (128, D)).T

    def q_block(b):
        P = {}
        for r in ORDER_B:
            P[r] = NT(unpack(wqtf[pl.ds(r * (dd // 2), dd // 2), :]), xform(r, b))
        o = [[None, None], [None, None]]
        for (i, k) in _quadrants(ORDER_B):
            zc = zcol[pl.ds(k * dd, dd), :]
            zc = jnp.concatenate([zc] * (tm // 128), axis=1)
            pq = phi(combine(P, GAMMA, i, k))
            t = (pq * zc).reshape(dd // DH, DH, tm)
            den = jnp.sum(t, axis=1, keepdims=True) + 1e-6
            o[k][i] = (pq.reshape(dd // DH, DH, tm) * (1.0 / den)).reshape(dd, tm)
        for r in range(R):
            of[pl.ds((b * R + r) * (dd // 2), dd // 2), :] = pack(form(ALPHA[r].T, o))

    def o_form2(sb, r, r2):
        nz = [(j2, i2) for j2 in range(2) for i2 in range(2) if ALPHA[r2].T[j2, i2]]
        if len(nz) == 1:
            (j2, i2), = nz
            return unpack(of[pl.ds(((2 * sb + i2) * R + r) * (dd // 2) + j2 * (dd // 4), dd // 4), :])
        return unpack(of2[pl.ds(((sb * R + r) * R + r2) * (dd // 4), dd // 4), :])

    def make_o_form2(sb, start):
        pacer = Pacer(start)
        for r in ORDER_A:
            for rc in range(4):
                z = pacer.tick(3)
                q4 = [[unpack(of[pl.ds(((2 * sb + i2) * R + r) * (dd // 2) + j2 * (dd // 4) + rc * 32, 32), :]).astype(f32)
                       for i2 in range(2)] for j2 in range(2)]
                zz = jnp.concatenate([jnp.concatenate([z] * 2, axis=1)] * 8, axis=0)
                q4[0][0] = q4[0][0] + zz
                q4[1][1] = q4[1][1] + zz
                for r2 in range(R):
                    if np.abs(ALPHA[r2]).sum() > 1:
                        of2[pl.ds(((sb * R + r) * R + r2) * (dd // 4) + rc * 32, 32), :] = pack(form(ALPHA[r2].T, q4))

    for b in range(NB - 1):
        q_block(b)

    idx = jnp.clip(jnp.max(idxf).astype(i32), 0, S - 1)
    i16 = pl.multiple_of((idx // 16) * 16, 16)
    x16 = x_v[pl.ds(i16, 16), :].astype(f32)
    mean16 = jnp.concatenate([st_mean[pl.ds(i16, 16), :]] * (D // 128), axis=1)
    inv16 = jnp.concatenate([st_inv[pl.ds(i16, 16), :]] * (D // 128), axis=1)
    xs = rnd((x16 - mean16) * inv16)
    rowm = lax.broadcasted_iota(i32, (16, D), 0) == (idx - i16)
    xrow = jnp.sum(jnp.where(rowm, xs, 0.0), axis=0, keepdims=True)
    xcol[...] = jnp.broadcast_to(xrow, (128, D)).T

    def matvec(w_ref, col_ref, nrows, c0, z):
        acc = None
        for i in range(nrows // 8):
            t = w_ref[pl.ds(8 * i, 8), pl.ds(c0, 128)].astype(f32) * col_ref[pl.ds(8 * i, 8), :]
            if i == 0 and z is not None:
                t = t + z
            acc = t if acc is None else acc + t
        return acc

    def pk_form(r):
        return unpack(pkf[pl.ds(r * (S // 4), S // 4), :])

    P = {}
    lhs = pk_form(ORDER_A[0]).T
    cwg.wait()
    cwu.wait()
    z = None
    for c in range(F // 128):
        ga = matvec(wg_v, xcol, D, c * 128, z)
        z = after(ga)
        ua = matvec(wu_v, xcol, D, c * 128, z)
        z = after(ua)
        gg = rnd(jnp.sum(ga, axis=0, keepdims=True))
        uu = rnd(jnp.sum(ua, axis=0, keepdims=True))
        hh = rnd(rnd(gg * jax.nn.sigmoid(gg)) * uu)
        hcol[pl.ds(c * 128, 128), :] = jnp.broadcast_to(hh, (128, 128)).T
    P[ORDER_A[0]] = NN(lhs, xform(ORDER_A[0]))
    for r in ORDER_A[1:4]:
        P[r] = TN(pk_form(r), xform(r))
    lhs = pk_form(ORDER_A[4]).T
    cwd.wait()
    cwv.wait()
    cwo.wait()
    z, ys = None, []
    for n in range(D // 128):
        ya = matvec(wd_v, hcol, F, n * 128, z)
        z = after(ya)
        ys.append(jnp.sum(ya, axis=0, keepdims=True))
    yy = jnp.where(rowm, jnp.concatenate(ys, axis=1) * jax.nn.sigmoid(rmax), 0.0)
    P[ORDER_A[4]] = NN(lhs, xform(ORDER_A[4]))
    for r in ORDER_A[5:]:
        P[r] = TN(pk_form(r), xform(r))

    zero = jnp.concatenate([after(ya)] * 16, axis=0)
    blk = lax.broadcasted_iota(i32, (128, 128), 0) // DH == lax.broadcasted_iota(i32, (128, 128), 1) // DH
    Mq = [None, None]
    for k in range(2):
        Gk = [combine(P, BETA_T, k, j) for j in range(2)]
        Ms = []
        for gi in range(dd // 128):
            g = k * (dd // 128) + gi
            Gg = jnp.concatenate([Gk[j][gi * 128:(gi + 1) * 128, :].astype(bf16) for j in range(2)], axis=1)
            kv = NN(Gg, wv_v[:, pl.ds(g * 128, 128)])
            kv = jnp.where(blk, kv, zero).astype(bf16)
            Ms.append(NN(kv, wo_v[pl.ds(g * 128, 128), :]))
        m_start = Ms[0][:8, :128]
        Mk = jnp.concatenate(Ms, axis=0)
        Mq[k] = [Mk[:, :dd], Mk[:, dd:]]
    for r in range(R):
        f1 = form(BETA[r], Mq)
        q4 = [[f1[j * (dd // 2):(j + 1) * (dd // 2), k * (dd // 2):(k + 1) * (dd // 2)] for k in range(2)] for j in range(2)]
        for r2 in range(R):
            mf[pl.ds((r * R + r2) * (dd // 4), dd // 4), :] = pack(form(BETA[r2], q4))

    make_o_form2(0, m_start)
    q_block(NB - 1)

    pending = []

    def send(r0, col0, ncol):
        off = pl.multiple_of(jnp.clip(i16 - r0, 0, TM - 16), 16) + r0
        inside = jnp.logical_and(i16 >= r0, i16 < r0 + TM)
        tile = out_v[pl.ds(off, 16), pl.ds(col0, ncol)].astype(f32) + jnp.where(inside, yy[:, col0:col0 + ncol], 0.0)
        out_v[pl.ds(off, 16), pl.ds(col0, ncol)] = tile.astype(bf16)
        c = copy(out_v.at[pl.ds(r0, TM), pl.ds(col0, ncol)], out_hbm.at[pl.ds(r0, TM), pl.ds(col0, ncol)])
        c.start()
        pending.append(c)

    def emit(b, i1, col0, Aq):
        for c in range(16):
            r0 = b * TM + c * 32 + i1 * 16
            xx = x_v[pl.ds(r0, 16), pl.ds(col0, dd // 2)].astype(f32)
            mean = jnp.concatenate([st_mean[pl.ds(r0, 16), :]] * (dd // 256), axis=1)
            inv = jnp.concatenate([st_inv[pl.ds(r0, 16), :]] * (dd // 256), axis=1)
            o = (Aq[c * 16:(c + 1) * 16, :] + xx) + (xx - mean) * inv
            out_v[pl.ds(r0, 16), pl.ds(col0, dd // 2)] = o.astype(bf16)

    for sb in range(NB // 2):
        last = sb == NB // 2 - 1
        Q, done = {}, set()
        for n, ro in enumerate(ORDER_B):
            P2 = {ri: TN(o_form2(sb, ri, ro), unpack(mf[pl.ds((ri * R + ro) * (dd // 4), dd // 4), :])) for ri in ORDER_A}
            Q[ro] = {q: combine(P2, GAMMA, *q) for q in [(1, 0), (0, 1), (0, 0), (1, 1)]}
            if n == 0 and not last:
                make_o_form2(sb + 1, Q[ro][1, 0][:8, :128])
            for (i2, k2) in [(1, 0), (0, 1), (0, 0), (1, 1)]:
                if (i2, k2) in done or not all(r in Q for r in range(R) if GAMMA[r][i2, k2]):
                    continue
                done.add((i2, k2))
                b = 2 * sb + i2
                fin = set()
                for (i1, k1) in _quadrants(ORDER_A):
                    emit(b, i1, k1 * dd + k2 * (dd // 2), combine({r: Q[r][i1, k1] for r in Q}, GAMMA, i2, k2))
                    fin.add((i1, k1))
                    if last and (1 - i1, k1) in fin:
                        send(b * TM, k1 * dd + k2 * (dd // 2), dd // 2)
                if not last and (i2, 1 - k2) in done:
                    send(b * TM, 0, D)
    for c in pending:
        c.wait()


@jax.jit
def pallas_parallel_sum__linear_attn_block__moe_arch_mod__prompt_kernel(
    A_x: jax.Array,
    A_wqkv: jax.Array,
    A_wo: jax.Array,
    B_x: jax.Array,
    B_w_r: jax.Array,
    B_w_gate: jax.Array,
    B_w_up: jax.Array,
    B_w_down: jax.Array,
):
    scratch = [
        pltpu.VMEM((S, D), bf16),
        pltpu.VMEM((D, D), bf16), pltpu.VMEM((D, D), bf16), pltpu.VMEM((D, D), bf16), pltpu.VMEM((D, D), bf16),
        pltpu.VMEM((8, 128), bf16),
        pltpu.VMEM((D, F), bf16), pltpu.VMEM((D, F), bf16), pltpu.VMEM((F, D), bf16),
        pltpu.VMEM((S, 128), f32), pltpu.VMEM((S, 128), f32),
        pltpu.VMEM((R * S // 4, dd), u32), pltpu.VMEM((R * S // 4, dd), u32),
        pltpu.VMEM((R * dd // 2, dd), u32), pltpu.VMEM((R * dd // 2, dd), u32),
        pltpu.VMEM((NB * R * dd // 2, tm), u32),
        pltpu.VMEM((R * R * dd // 4, dd // 2), u32),
        pltpu.VMEM((D, 128), f32),
        pltpu.VMEM((S, D), bf16),
        pltpu.VMEM((D, 128), f32), pltpu.VMEM((F, 128), f32),
        pltpu.VMEM((2 * R * R * dd // 4, tm), u32),
        pltpu.SemaphoreType.DMA((25,)),
    ]
    any_spec = pl.BlockSpec(memory_space=pl.ANY)
    out = pl.pallas_call(
        _kernel,
        out_shape=jax.ShapeDtypeStruct((S, D), bf16),
        in_specs=[any_spec] * 7,
        out_specs=any_spec,
        scratch_shapes=scratch,
        compiler_params=pltpu.CompilerParams(
            vmem_limit_bytes=120 * 1024 * 1024,
            flags={"XLA_TPU_EVENLY_DISTRIBUTE_CRITICAL_NODES": True}),
    )(A_x.reshape(S, D), A_wqkv, A_wo, B_w_r.reshape(8, 128), B_w_gate, B_w_up, B_w_down)
    return out.reshape(1, S, D)
```
